```python
import jax
import jax.numpy as jnp

def _softmax(x, axis=-1):
    return jax.nn.softmax(x, axis=axis)

def _gelu(x):
    return jax.nn.gelu(x, approximate=True)

def _silu(x):
    return jax.nn.silu(x)

def _sigmoid(x):
    return jax.nn.sigmoid(x)

def _layernorm(x, axis=-1, eps=1e-05):
    m = jnp.mean(x, axis=axis, keepdims=True)
    v = jnp.var(x, axis=axis, keepdims=True)
    return (x - m) / jnp.sqrt(v + eps)

def _scatter_add(tgt, idx, src, axis=0):
    return tgt.at[idx].add(src)

def _segment_sum(src, seg, n):
    return jax.ops.segment_sum(src, seg, n)

class _Rng:

    def __init__(self, key):
        self._k = key

    def _next(self):
        self._k, sub = jax.random.split(self._k)
        return sub

    def normal(self, shape):
        return jax.random.normal(self._next(), shape, dtype=jnp.bfloat16)

    def randint(self, lo, hi, shape):
        return jax.random.randint(self._next(), shape, lo, hi, dtype=jnp.int32)

    def uniform(self, shape, lo=0.0, hi=1.0):
        return jax.random.uniform(self._next(), shape, jnp.bfloat16, lo, hi)

    def permutation(self, n):
        return jax.random.permutation(self._next(), n)
kernel_name = 'gated_mix__memory_aug_recurrent_mem_tr__spectral_gfnet__prompt'

def setup_inputs():
    _rng = _Rng(jax.random.key(int.from_bytes(__import__("os").urandom(4), "little")))
    _w = lambda a: (lambda t: t.astype(jnp.bfloat16) if jnp.issubdtype(t.dtype, jnp.floating) else t)(jnp.asarray(a))

    def _A_setup():
        B, S, Dm = (1, 2048, 1024)
        H, Dh = (32, 128)
        M, seg = (8, 32)
        seg = min(seg, S)
        S = S // seg * seg
        return {'x': _w((lambda *s: _rng.normal(s) * 0.05)(B, S, Dm)), 'mem0': _w((lambda *s: _rng.normal(s) * 0.05)(B, M, Dm)), 'Wq': _w((lambda *s: _rng.normal(s) * 0.05)(Dm, H, Dh) * Dm ** (-0.5)), 'Wk': _w((lambda *s: _rng.normal(s) * 0.05)(Dm, H, Dh) * Dm ** (-0.5)), 'Wv': _w((lambda *s: _rng.normal(s) * 0.05)(Dm, H, Dh) * Dm ** (-0.5)), 'Wo': _w((lambda *s: _rng.normal(s) * 0.05)(H, Dh, Dm) * (H * Dh) ** (-0.5)), 'seg_len': seg}
    _A_in = _A_setup()

    def _B_setup():
        B, S, D = (1, 2048, 1024)
        Df = D // 2 + 1
        return {'x': _w((lambda *s: _rng.normal(s) * 0.05)(B, S, D)), 'w_r': _w((lambda *s: _rng.normal(s) * 0.05)(S, Df) * 0.02), 'w_i': _w((lambda *s: _rng.normal(s) * 0.05)(S, Df) * 0.02)}
    _B_in = _B_setup()
    return {'A_x': _A_in['x'], 'A_mem0': _A_in['mem0'], 'A_Wq': _A_in['Wq'], 'A_Wk': _A_in['Wk'], 'A_Wv': _A_in['Wv'], 'A_Wo': _A_in['Wo'], 'A_seg_len': _A_in['seg_len'], 'B_x': _B_in['x'], 'B_w_r': _B_in['w_r'], 'B_w_i': _B_in['w_i'], 'gate_w': _w((lambda *s: _rng.normal(s) * 0.05)(1024))}

def reference(A_x, A_mem0, A_Wq, A_Wk, A_Wv, A_Wo, A_seg_len, B_x, B_w_r, B_w_i, gate_w):

    def _A_ref(x, mem0, Wq, Wk, Wv, Wo, seg_len):
        B, S, Dm = x.shape
        H, Dh = (Wq.shape[1], Wq.shape[2])
        M = mem0.shape[1]
        scale = Dh ** (-0.5)
        n_seg = S // seg_len
        L = M + seg_len
        idx = jnp.arange(L)
        mask = (idx[:, None] < M) | (idx[:, None] >= idx[None, :])
        mem = mem0
        outs = []
        for s in range(n_seg):
            xs = x[:, s * seg_len:(s + 1) * seg_len, :].copy()
            h = jnp.concatenate([mem, xs], axis=1)
            q = jnp.einsum('btd,dhe->bhte', h, Wq)
            k = jnp.einsum('btd,dhe->bhte', h, Wk)
            v = jnp.einsum('btd,dhe->bhte', h, Wv)
            scores = jnp.einsum('bhqe,bhke->bhqk', q, k) * scale
            scores = jnp.where(mask[None, None], scores, -1000000000.0)
            p = _softmax(scores, axis=-1)
            o = jnp.einsum('bhqk,bhke->bhqe', p, v)
            o = jnp.einsum('bhte,hed->btd', o, Wo)
            mem = o[:, :M, :].copy()
            outs.append(o[:, M:, :])
        return jnp.concatenate(outs, axis=1)

    def _B_ref(x, w_r, w_i):
        B, S, D = x.shape
        X = (lambda x, axes=(-2, -1): jnp.fft.rfft2(x.astype(jnp.float32), axes=axes))(x, axes=(-2, -1))
        W = w_r + 1j * w_i
        X = X * W
        y = (lambda x, s, axes=(-2, -1): jnp.fft.irfft2(x, s=s, axes=axes).astype(jnp.bfloat16))(X, (S, D), axes=(-2, -1))
        return y
    x = A_x
    g = _sigmoid((x * gate_w).sum(-1, keepdims=True))
    a = _A_ref(x, A_mem0, A_Wq, A_Wk, A_Wv, A_Wo, A_seg_len)
    b = _B_ref(x, B_w_r, B_w_i)
    return g * a + (1 - g) * b
```

```python
import functools

import jax
import jax.numpy as jnp
import numpy as np
import jax.experimental.pallas as pl
import jax.experimental.pallas.tpu as pltpu

f32 = jnp.float32
bf16 = jnp.bfloat16
u32 = jnp.uint32
i32 = jnp.int32

S, D, H, DH, M, SEG = 2048, 1024, 32, 128, 8, 32
L = M + SEG
NSEG = S // SEG
KR = 520


def _bf16_bits(a):
    u = np.ascontiguousarray(a, dtype=np.float32).view(np.uint32).astype(np.uint64)
    return ((u + 0x7FFF + ((u >> 16) & 1)) >> 16).astype(np.uint32)


def _pack_rows(a):
    b = _bf16_bits(a)
    return (b[..., 0::2, :] | (b[..., 1::2, :] << 16)).astype(np.uint32)


def _build_consts():
    b = np.arange(128)
    r = np.arange(64)

    def cs(k):
        ang = 2 * np.pi * (np.outer(k, b) % D) / D
        return np.cos(ang), np.sin(ang)

    mats = []
    for j in (1, 2, 3):
        k = np.concatenate([j + 8 * r, 8 - j + 8 * r])
        c, s = cs(k)
        sg = np.concatenate([-np.ones(64), np.ones(64)])[:, None]
        mats.append(np.block([[c, sg * s], [-s, sg * c]]))
    sc = 1.0 / (D * S)
    k0 = np.concatenate([8 * r, 4 + 8 * r])
    c, s = cs(k0)
    g0 = np.zeros((256, 256))
    cf = np.full(128, 2.0)
    cf[0] = 1.0
    g0[0:64, 0:128] = c[0:64] * cf[0:64, None]
    g0[64:128, 128:256] = 2 * c[64:128]
    g0[128:192, 0:128] = -2 * s[0:64]
    g0[128, 0:128] = (-1.0) ** b
    g0[192:256, 128:256] = -2 * s[64:128]
    mats.append(g0 * sc)
    for j in (1, 2, 3):
        k = np.concatenate([j + 8 * r, 8 - j + 8 * r])
        c, s = cs(k)
        tau = np.concatenate([np.ones(64), -np.ones(64)])[:, None]
        mats.append(np.block([[2 * c, 2 * tau * s], [-2 * s, 2 * tau * c]]) * sc)
    n2 = np.arange(128)
    for n1 in range(16):
        ang = 2 * np.pi * (np.outer(n1 + 16 * n2, n2) % S) / S
        mr, mi = np.cos(ang), -np.sin(ang)
        mats.append(np.block([[mr, mi], [-mi, mr]]))
    cu = _pack_rows(np.stack(mats))
    c0, s0 = cs(8 * r)
    c4, s4 = cs(4 + 8 * r)
    a0 = np.zeros((136, 128))
    a0[0:64] = c0
    a0[64:128] = -s0
    a0[128] = (-1.0) ** b
    a4 = np.concatenate([c4, -s4])
    cf32 = np.concatenate([a0, a4]).astype(np.float32)
    return cu, cf32


_CU, _CF = _build_consts()
_C_A, _C_G, _C_M = 0, 3, 7


def _dot(a, b):
    return jax.lax.dot_general(a, b, (((1,), (0,)), ((), ())), preferred_element_type=f32)


def _dot_nt(a, b):
    return jax.lax.dot_general(a, b, (((1,), (1,)), ((), ())), preferred_element_type=f32)


def _lo(w):
    return pltpu.bitcast(w << 16, f32)


def _hi(w):
    return pltpu.bitcast(w & jnp.uint32(0xFFFF0000), f32)


def _bf16_word(x):
    return pltpu.bitcast(x.astype(bf16).astype(f32), u32)


_R2 = float(np.sqrt(0.5))


def _cmul_const(z, ang):
    zr, zi = z
    c, s = float(np.cos(ang)), float(np.sin(ang))
    q = int(round(ang / (np.pi / 4)))
    if abs(ang - q * np.pi / 4) < 1e-9:
        q %= 8
        if q == 0:
            return zr, zi
        if q == 2:
            return -zi, zr
        if q == 4:
            return -zr, -zi
        if q == 6:
            return zi, -zr
        if q == 1:
            return (zr - zi) * _R2, (zr + zi) * _R2
        if q == 3:
            return (zr + zi) * (-_R2), (zr - zi) * _R2
        if q == 5:
            return (zi - zr) * _R2, (zr + zi) * (-_R2)
        return (zr + zi) * _R2, (zi - zr) * _R2
    return zr * c - zi * s, zr * s + zi * c


def _add(a, b):
    return a[0] + b[0], a[1] + b[1]


def _sub(a, b):
    return a[0] - b[0], a[1] - b[1]


def _bfly4(x0, x1, x2, x3, sign):
    s0, s1 = _add(x0, x2), _sub(x0, x2)
    s2, s3 = _add(x1, x3), _sub(x1, x3)
    y0, y2 = _add(s0, s2), _sub(s0, s2)
    if sign < 0:
        y1 = (s1[0] + s3[1], s1[1] - s3[0])
        y3 = (s1[0] - s3[1], s1[1] + s3[0])
    else:
        y1 = (s1[0] - s3[1], s1[1] + s3[0])
        y3 = (s1[0] + s3[1], s1[1] - s3[0])
    return y0, y1, y2, y3


def _fft16(x, sign):
    t = [[None] * 4 for _ in range(4)]
    for b in range(4):
        y = _bfly4(x[b], x[4 + b], x[8 + b], x[12 + b], sign)
        for c in range(4):
            t[c][b] = _cmul_const(y[c], sign * 2 * np.pi * b * c / 16)
    out = [None] * 16
    for c in range(4):
        y = _bfly4(t[c][0], t[c][1], t[c][2], t[c][3], sign)
        for d in range(4):
            out[c + 4 * d] = y[d]
    return out


def _kernel(x_hbm, mem0_ref, wq_hbm, wk_hbm, wv_hbm, wo_hbm, wrt_hbm, wit_hbm, gw_ref, cu_hbm, cf_hbm,
            out_hbm,
            xu, wraw, wqkv, wo2, cu, cf, wu, wny, tr, ti, bu, h_ref, o_ref, ob, sems, osem):
    def start(cs):
        for c in cs:
            c.start()

    def wait(cs):
        for c in cs:
            c.wait()

    xw = x_hbm.bitcast(u32)
    c_x = [pltpu.make_async_copy(xw.at[:, 128 * a:128 * (a + 1)], xu.at[a], sems.at[0]) for a in range(8)]
    c_c = [pltpu.make_async_copy(cu_hbm, cu, sems.at[1]), pltpu.make_async_copy(cf_hbm, cf, sems.at[1])]
    c_w = []
    for t, w in enumerate((wrt_hbm, wit_hbm)):
        ww = w.at[0:512].bitcast(u32)
        c_w += [pltpu.make_async_copy(ww.at[:, 128 * k:128 * (k + 1)], wu.at[t, k], sems.at[2]) for k in range(16)]
        c_w.append(pltpu.make_async_copy(w.at[512:513], wny.at[t], sems.at[2]))
    c_qkv = []
    for t, w in enumerate((wq_hbm, wk_hbm, wv_hbm)):
        ww = w.bitcast(u32)
        c_qkv.append([pltpu.make_async_copy(ww.at[:, i, :], wraw.at[t, i], sems.at[3 + t]) for i in range(16)])
    wow = wo_hbm.bitcast(u32)
    c_o = [pltpu.make_async_copy(wow.at[:, :, 128 * j:128 * (j + 1)], wo2.at[j], sems.at[6]) for j in range(8)]
    start(c_x)
    start(c_c)
    start(c_w)
    for c in c_qkv:
        start(c)
    start(c_o)

    lane = jax.lax.broadcasted_iota(i32, (128, 128), 1)

    def cmat(i):
        return pltpu.bitcast(cu[i], bf16)

    wait(c_x)
    wait(c_c)

    def fwd(i, carry):
        xw_t = [xu[a, pl.ds(i, 128, stride=8), :] for a in range(8)]
        for half in range(2):
            n1 = 2 * i + half
            x = [(_lo if half == 0 else _hi)(w) for w in xw_t]
            a0, a1, a2, a3 = x[0] + x[4], x[1] + x[5], x[2] + x[6], x[3] + x[7]
            d0, d1, d2, d3 = x[0] - x[4], x[1] - x[5], x[2] - x[6], x[3] - x[7]
            e0, e1 = a0 + a2, a1 + a3
            u, w = (d1 - d3) * _R2, (d1 + d3) * _R2
            p0, p4 = e0 + e1, e0 - e1
            planes = [(d0 + u, d2 + w), (a0 - a2, a1 - a3), (d0 - u, w - d2)]
            o0 = _dot_nt(cf[0:136, :], p0)
            o4 = _dot_nt(cf[136:264, :], p4)
            oj = [_dot_nt(cmat(_C_A + j), jnp.concatenate(planes[j], axis=1)) for j in range(3)]
            xr = jnp.concatenate([o0[0:64], o4[0:64]] + [o[0:128] for o in oj] + [o0[128:136]], axis=0)
            xi = jnp.concatenate([o0[64:128], o4[64:128]] + [o[128:256] for o in oj]
                                 + [jnp.zeros((8, 128), f32)], axis=0)
            t = _dot(jnp.concatenate([xr, xi], axis=1), cmat(_C_M + n1))
            c0 = pl.multiple_of(n1 * 128, 128)
            tr[0:KR, pl.ds(c0, 128)] = t[:, 0:128]
            ti[0:KR, pl.ds(c0, 128)] = t[:, 128:256]
        return carry

    jax.lax.fori_loop(0, 8, fwd, 0)

    wait(c_w)

    def mid_group(r0, wr_fn, wi_fn):
        z = [(tr[pl.ds(r0, 8), 128 * n:128 * (n + 1)], ti[pl.ds(r0, 8), 128 * n:128 * (n + 1)]) for n in range(16)]
        z = _fft16(z, -1)
        q = []
        for k in range(16):
            wr, wi = wr_fn(k), wi_fn(k)
            zr, zi = z[k]
            q.append((zr * wr - zi * wi, zr * wi + zi * wr))
        z = _fft16(q, +1)
        for n in range(16):
            tr[pl.ds(r0, 8), 128 * n:128 * (n + 1)] = z[n][0]
            ti[pl.ds(r0, 8), 128 * n:128 * (n + 1)] = z[n][1]

    for blk, half, res in ((0, 0, 0), (0, 1, 4), (1, 0, 1), (1, 1, 7), (2, 0, 2), (2, 1, 6), (3, 0, 3), (3, 1, 5)):
        sel = _lo if res % 2 == 0 else _hi

        def mid(g, carry, blk=blk, half=half, res=res, sel=sel):
            r0 = pl.multiple_of(128 * blk + 64 * half + 8 * g, 8)
            p0 = res // 2 + 32 * g
            mid_group(r0,
                      lambda k: sel(wu[0, k, pl.ds(p0, 8, stride=4), :]),
                      lambda k: sel(wu[1, k, pl.ds(p0, 8, stride=4), :]))
            return carry

        jax.lax.fori_loop(0, 8, mid, 0)
    mid_group(512,
              lambda k: jnp.broadcast_to(wny[0, :, 128 * k:128 * (k + 1)].astype(f32), (8, 128)),
              lambda k: jnp.broadcast_to(wny[1, :, 128 * k:128 * (k + 1)].astype(f32), (8, 128)))

    def inv(i, carry):
        ys = []
        for half in range(2):
            n1 = 2 * i + half
            c0 = pl.multiple_of(n1 * 128, 128)
            ms = cmat(_C_M + n1)
            zc = jnp.concatenate([tr[0:512, pl.ds(c0, 128)], ti[0:512, pl.ds(c0, 128)]], axis=1)
            z = _dot_nt(ms, zc)
            zn = jnp.concatenate([tr[512:640, pl.ds(c0, 128)], ti[512:640, pl.ds(c0, 128)]], axis=1)
            ny = _dot_nt(ms[0:128], zn)
            zr, zi = z[0:128], z[128:256]
            zi0 = jnp.where(lane == 0, ny, zi[:, 0:128])
            u = _dot(jnp.concatenate([zr[:, 0:128], zi0], axis=1), cmat(_C_G))
            v = [_dot(jnp.concatenate([zr[:, 128 * j:128 * (j + 1)], zi[:, 128 * j:128 * (j + 1)]], axis=1),
                      cmat(_C_G + j)) for j in (1, 2, 3)]
            u0, u4 = u[:, 0:128], u[:, 128:256]
            v1r, v1i = v[0][:, 0:128], v[0][:, 128:256]
            v2r, v2i = v[1][:, 0:128], v[1][:, 128:256]
            v3r, v3i = v[2][:, 0:128], v[2][:, 128:256]
            e, o = u0 + u4, u0 - u4
            ep, em = e + v2r, e - v2r
            sa, da = v1r + v3r, v1r - v3r
            di, si = v1i - v3i, v1i + v3i
            p, q = (da - si) * _R2, (da + si) * _R2
            om, op = o - v2i, o + v2i
            ys.append([ep + sa, om + p, em - di, op - q, ep - sa, om - p, em + di, op + q])
        for a in range(8):
            bu[a, pl.ds(i, 128, stride=8), :] = (_bf16_word(ys[0][a]) >> 16) | _bf16_word(ys[1][a])
        return carry

    jax.lax.fori_loop(0, 8, inv, 0)

    for t in range(3):
        wait(c_qkv[t])

        def rep(i, carry, t=t):
            ev = wraw[t, i, pl.ds(0, 512, stride=2), :]
            od = wraw[t, i, pl.ds(1, 512, stride=2), :]
            wqkv[2 * i, :, 128 * t:128 * (t + 1)] = (ev & jnp.uint32(0xFFFF)) | (od << 16)
            wqkv[2 * i + 1, :, 128 * t:128 * (t + 1)] = (ev >> 16) | (od & jnp.uint32(0xFFFF0000))
            return carry

        jax.lax.fori_loop(0, 16, rep, 0)
    wait(c_o)

    h_ref[0:M, :] = mem0_ref[...].astype(f32)
    row = jax.lax.broadcasted_iota(i32, (L, L), 0)
    col = jax.lax.broadcasted_iota(i32, (L, L), 1)
    mask = (row < M) | (row >= col)
    scale = DH ** -0.5

    def step(s, carry):
        r0 = pl.multiple_of(s * SEG, SEG)
        p0 = pl.multiple_of(s * (SEG // 2), SEG // 2)
        for a in range(8):
            h_ref[M:L, 128 * a:128 * (a + 1)] = pltpu.bitcast(xu[a, pl.ds(p0, SEG // 2), :], bf16).astype(f32)
        st = {}
        for it in range(H + 2):
            if it < H:
                st[it] = dict(qkv=_dot(h_ref[...], pltpu.bitcast(wqkv[it], bf16)))
            a = it - 1
            if 0 <= a < H:
                qkv = st[a]['qkv']
                st[a]['sc'] = _dot_nt(qkv[:, 0:128], qkv[:, 128:256])
            b = it - 2
            if 0 <= b < H:
                o_ref[:, b * 128:(b + 1) * 128] = _dot(st[b]['p'], st[b]['qkv'][:, 256:384]) / st[b]['l']
                del st[b]
            if 0 <= a < H:
                sc = jnp.where(mask, st[a]['sc'] * scale, -1e9)
                p = jnp.exp(sc - jnp.max(sc, axis=-1, keepdims=True))
                st[a]['p'] = p
                st[a]['l'] = jnp.sum(p, axis=-1, keepdims=True)
        gw = gw_ref[...].astype(f32)
        z = jnp.sum(h_ref[M:L, :] * gw, axis=-1, keepdims=True)
        g = jax.nn.sigmoid(z)
        o = o_ref[...]
        for j in range(8):
            r = _dot(o, pltpu.bitcast(wo2[j].reshape(2048, 128), bf16))
            h_ref[0:M, 128 * j:128 * (j + 1)] = r[0:M]
            bb = pltpu.bitcast(bu[j, pl.ds(p0, SEG // 2), :], bf16).astype(f32)
            ob[pl.ds(r0, SEG), 128 * j:128 * (j + 1)] = (bb + g * (r[M:L] - bb)).astype(bf16)
        pltpu.make_async_copy(ob.at[pl.ds(r0, SEG)], out_hbm.at[pl.ds(r0, SEG)], osem).start()
        return carry

    jax.lax.fori_loop(0, NSEG, step, 0)

    def drain(s, carry):
        pltpu.make_async_copy(ob.at[pl.ds(0, SEG)], out_hbm.at[pl.ds(0, SEG)], osem).wait()
        return carry

    jax.lax.fori_loop(0, NSEG, drain, 0)


@functools.partial(jax.jit, static_argnames=("A_seg_len",))
def pallas_gated_mix__memory_aug_recurrent_mem_tr__spectral_gfnet__prompt_kernel(
    A_x, A_mem0, A_Wq, A_Wk, A_Wv, A_Wo, A_seg_len, B_x, B_w_r, B_w_i, gate_w,
):
    del B_x
    assert A_x.shape == (1, S, D) and A_mem0.shape == (1, M, D) and A_Wq.shape == (D, H, DH)
    assert int(A_seg_len) == SEG
    V = pltpu.VMEM
    hbm = pl.BlockSpec(memory_space=pltpu.MemorySpace.HBM)
    vm = pl.BlockSpec(memory_space=pltpu.MemorySpace.VMEM)
    out = pl.pallas_call(
        _kernel,
        out_shape=jax.ShapeDtypeStruct((S, D), bf16),
        in_specs=[hbm, vm, hbm, hbm, hbm, hbm, hbm, hbm, vm, hbm, hbm],
        out_specs=hbm,
        scratch_shapes=[
            V((8, S // 2, 128), u32),
            V((3, 16, D, 128), u32),
            V((H, D // 2, 384), u32),
            V((8, H, DH // 2, 128), u32),
            V(_CU.shape, u32),
            V(_CF.shape, f32),
            V((2, 16, 256, 128), u32),
            V((2, 1, S), bf16),
            V((640, S), f32),
            V((640, S), f32),
            V((8, S // 2, 128), u32),
            V((L, D), f32),
            V((L, H * DH), f32),
            V((S, D), bf16),
            pltpu.SemaphoreType.DMA((7,)),
            pltpu.SemaphoreType.DMA,
        ],
        compiler_params=pltpu.CompilerParams(vmem_limit_bytes=112 * 1024 * 1024),
    )(A_x.reshape(S, D), A_mem0.reshape(M, D), A_Wq, A_Wk, A_Wv, A_Wo,
      B_w_r.T, B_w_i.T, gate_w.reshape(1, D), _CU, _CF)
    return out.reshape(1, S, D)
```

```python
import functools

import jax
import jax.numpy as jnp
import numpy as np
import jax.experimental.pallas as pl
import jax.experimental.pallas.tpu as pltpu

f32 = jnp.float32
bf16 = jnp.bfloat16
u32 = jnp.uint32
i32 = jnp.int32

S, D, H, DH, M, SEG = 2048, 1024, 32, 128, 8, 32
L = M + SEG
NSEG = S // SEG
WO_AT = 5
UNROLL = 3
LAGQ, LAGP = 1, 3
KS = 28
XAT = 8
KR = 520


_C_A, _C_G = 0, 3


def _dot(a, b):
    return jax.lax.dot_general(a, b, (((1,), (0,)), ((), ())), preferred_element_type=f32)


def _dot_nt(a, b):
    return jax.lax.dot_general(a, b, (((1,), (1,)), ((), ())), preferred_element_type=f32)


def _lo(w):
    return pltpu.bitcast(w << 16, f32)


def _hi(w):
    return pltpu.bitcast(w & jnp.uint32(0xFFFF0000), f32)


def _bf16_word(x):
    return pltpu.bitcast(x.astype(bf16).astype(f32), u32)


_R2 = float(np.sqrt(0.5))


def _cmul_const(z, ang):
    zr, zi = z
    c, s = float(np.cos(ang)), float(np.sin(ang))
    q = int(round(ang / (np.pi / 4)))
    if abs(ang - q * np.pi / 4) < 1e-9:
        q %= 8
        if q == 0:
            return zr, zi
        if q == 2:
            return -zi, zr
        if q == 4:
            return -zr, -zi
        if q == 6:
            return zi, -zr
        if q == 1:
            return (zr - zi) * _R2, (zr + zi) * _R2
        if q == 3:
            return (zr + zi) * (-_R2), (zr - zi) * _R2
        if q == 5:
            return (zi - zr) * _R2, (zr + zi) * (-_R2)
        return (zr + zi) * _R2, (zi - zr) * _R2
    return zr * c - zi * s, zr * s + zi * c


def _add(a, b):
    return a[0] + b[0], a[1] + b[1]


def _sub(a, b):
    return a[0] - b[0], a[1] - b[1]


def _bfly4(x0, x1, x2, x3, sign):
    s0, s1 = _add(x0, x2), _sub(x0, x2)
    s2, s3 = _add(x1, x3), _sub(x1, x3)
    y0, y2 = _add(s0, s2), _sub(s0, s2)
    if sign < 0:
        y1 = (s1[0] + s3[1], s1[1] - s3[0])
        y3 = (s1[0] - s3[1], s1[1] + s3[0])
    else:
        y1 = (s1[0] - s3[1], s1[1] + s3[0])
        y3 = (s1[0] + s3[1], s1[1] - s3[0])
    return y0, y1, y2, y3


def _fft16(x, sign):
    t = [[None] * 4 for _ in range(4)]
    for b in range(4):
        y = _bfly4(x[b], x[4 + b], x[8 + b], x[12 + b], sign)
        for c in range(4):
            t[c][b] = _cmul_const(y[c], sign * 2 * np.pi * b * c / 16)
    out = [None] * 16
    for c in range(4):
        y = _bfly4(t[c][0], t[c][1], t[c][2], t[c][3], sign)
        for d in range(4):
            out[c + 4 * d] = y[d]
    return out


def _kernel(x_hbm, mem0_hbm, wq_hbm, wk_hbm, wv_hbm, wo_hbm, wrt_hbm, wit_hbm, gw_hbm,
            out_hbm,
            mem0_ref, gw_ref, xu, wraw, wqkv, wo2, cu, ca, ms, wu, wny, tr, ti, bu, h_ref, o_ref, part_ref, ob, sems, qsem, wsem, osem):
    def start(cs):
        for c in cs:
            c.start()

    def wait(cs):
        for c in cs:
            c.wait()

    c_x = [pltpu.make_async_copy(x_hbm, ob, sems.at[0])]
    c_w = []
    for t, w in enumerate((wrt_hbm, wit_hbm)):
        ww = w.at[0:512].bitcast(u32)
        c_w += [pltpu.make_async_copy(ww.at[:, 128 * k:128 * (k + 1)], wu.at[t, k], sems.at[1]) for k in range(16)]
        c_w.append(pltpu.make_async_copy(w.at[512:513], wny.at[t], sems.at[1]))
    c_qkv = [[pltpu.make_async_copy(w.bitcast(u32).at[:, i, :], wraw.at[t, i], qsem.at[i])
              for t, w in enumerate((wq_hbm, wk_hbm, wv_hbm))] for i in range(16)]
    wow = wo_hbm.bitcast(u32)
    c_o = [pltpu.make_async_copy(wow.at[8 * q:8 * q + 8, :, 512 * hf:512 * (hf + 1)], wo2.at[hf, 8 * q:8 * q + 8],
                                 wsem.at[4 * hf + q]) for hf in range(2) for q in range(4)]
    c_p = [pltpu.make_async_copy(mem0_hbm, mem0_ref, sems.at[2]), pltpu.make_async_copy(gw_hbm, gw_ref, sems.at[2])]
    start(c_x)
    start(c_p)
    start(c_w)

    lane = jax.lax.broadcasted_iota(i32, (128, 128), 1)

    def cmat(i):
        return pltpu.bitcast(cu[i], bf16)

    rowi = jax.lax.broadcasted_iota(i32, (128, 128), 0)
    first = rowi < 64
    gscale = 1.0 / (D * S)

    def pack(m):
        return pltpu.bitcast(m.astype(bf16), u32)

    def blk2(a, b, c, d):
        return jnp.concatenate([jnp.concatenate([a, b], axis=1), jnp.concatenate([c, d], axis=1)], axis=0)

    alt = jnp.where((lane & 1) == 0, 1.0, -1.0).astype(f32)
    for j in range(4):
        lo, hi = (0, 4) if j == 0 else (j, 8 - j)
        k = jnp.where(first, lo + 8 * rowi, hi + 8 * (rowi - 64))
        ang = ((k * lane) & (D - 1)).astype(f32) * (2 * np.pi / D)
        c, s = jnp.cos(ang), jnp.sin(ang)
        if j == 0:
            ca[0:64, :] = c[0:64]
            ca[64:128, :] = -s[0:64]
            ca[128:136, :] = jnp.where(rowi[0:8] == 0, alt[0:8], 0.0)
            ca[136:200, :] = c[64:128]
            ca[200:264, :] = -s[64:128]
            c2 = jnp.where(rowi == 0, c, 2.0 * c) * gscale
            s2 = jnp.where(rowi == 0, alt, -2.0 * s) * gscale
            cu[_C_G] = pack(blk2(jnp.where(first, c2, 0.0), jnp.where(first, 0.0, c2),
                                 jnp.where(first, s2, 0.0), jnp.where(first, 0.0, s2)))
        else:
            sg = jnp.where(first, -s, s)
            cg = jnp.where(first, -c, c)
            cu[_C_A + j - 1] = pack(blk2(c, sg, -s, cg))
            cu[_C_G + j] = pack(blk2(2.0 * gscale * c, -2.0 * gscale * sg, -2.0 * gscale * s, -2.0 * gscale * cg))
    ang = ((rowi * lane) & 127).astype(f32) * (2 * np.pi / 128)
    ca[264:392, :] = jnp.cos(ang)
    ca[392:520, :] = -jnp.sin(ang)
    tr[KR:, :] = jnp.zeros((640 - KR, S), f32)
    ti[KR:, :] = jnp.zeros((640 - KR, S), f32)

    def gen_ms(n1, carry):
        fr, fi = ca[264:392, :], ca[392:520, :]
        ang = (n1 * lane[0:8]).astype(f32) * (2 * np.pi / S)
        t_r = jnp.broadcast_to(jnp.cos(ang)[0:1], (128, 128))
        t_i = jnp.broadcast_to(-jnp.sin(ang)[0:1], (128, 128))
        mr, mi = fr * t_r - fi * t_i, fr * t_i + fi * t_r
        ms[n1] = pack(blk2(mr, mi, -mi, mr))
        return carry

    jax.lax.fori_loop(0, 16, gen_ms, 0)
    wait(c_x)
    for c in c_qkv:
        start(c)

    def split_x(c, carry):
        r0 = pl.multiple_of(c * 128, 128)
        for a in range(8):
            xu[a, pl.ds(pl.multiple_of(c * 64, 64), 64), :] = pltpu.bitcast(ob[pl.ds(r0, 128), 128 * a:128 * (a + 1)], u32)
        return carry

    jax.lax.fori_loop(0, 16, split_x, 0)

    def fwd(i, carry):
        xw_t = [xu[a, pl.ds(i, 128, stride=8), :] for a in range(8)]
        for half in range(2):
            n1 = 2 * i + half
            x = [(_lo if half == 0 else _hi)(w) for w in xw_t]
            a0, a1, a2, a3 = x[0] + x[4], x[1] + x[5], x[2] + x[6], x[3] + x[7]
            d0, d1, d2, d3 = x[0] - x[4], x[1] - x[5], x[2] - x[6], x[3] - x[7]
            e0, e1 = a0 + a2, a1 + a3
            u, w = (d1 - d3) * _R2, (d1 + d3) * _R2
            p0, p4 = e0 + e1, e0 - e1
            planes = [(d0 + u, d2 + w), (a0 - a2, a1 - a3), (d0 - u, w - d2)]
            o0 = _dot_nt(ca[0:136, :], p0)
            o4 = _dot_nt(ca[136:264, :], p4)
            oj = [_dot_nt(cmat(_C_A + j), jnp.concatenate(planes[j], axis=1)) for j in range(3)]
            xr = jnp.concatenate([o0[0:64], o4[0:64]] + [o[0:128] for o in oj] + [o0[128:136]], axis=0)
            xi = jnp.concatenate([o0[64:128], o4[64:128]] + [o[128:256] for o in oj]
                                 + [jnp.zeros((8, 128), f32)], axis=0)
            t = _dot(jnp.concatenate([xr, xi], axis=1), pltpu.bitcast(ms[n1], bf16))
            c0 = pl.multiple_of(n1 * 128, 128)
            tr[0:KR, pl.ds(c0, 128)] = t[:, 0:128]
            ti[0:KR, pl.ds(c0, 128)] = t[:, 128:256]
        return carry

    jax.lax.fori_loop(0, 8, fwd, 0)

    wait(c_w)

    def mid_group(r0, wr_fn, wi_fn):
        z = [(tr[pl.ds(r0, 8), 128 * n:128 * (n + 1)], ti[pl.ds(r0, 8), 128 * n:128 * (n + 1)]) for n in range(16)]
        z = _fft16(z, -1)
        q = []
        for k in range(16):
            wr, wi = wr_fn(k), wi_fn(k)
            zr, zi = z[k]
            q.append((zr * wr - zi * wi, zr * wi + zi * wr))
        z = _fft16(q, +1)
        for n in range(16):
            tr[pl.ds(r0, 8), 128 * n:128 * (n + 1)] = z[n][0]
            ti[pl.ds(r0, 8), 128 * n:128 * (n + 1)] = z[n][1]

    for blk, half, res in ((0, 0, 0), (0, 1, 4), (1, 0, 1), (1, 1, 7), (2, 0, 2), (2, 1, 6), (3, 0, 3), (3, 1, 5)):
        sel = _lo if res % 2 == 0 else _hi

        def mid(g, carry, blk=blk, half=half, res=res, sel=sel):
            r0 = pl.multiple_of(128 * blk + 64 * half + 8 * g, 8)
            p0 = res // 2 + 32 * g
            mid_group(r0,
                      lambda k: sel(wu[0, k, pl.ds(p0, 8, stride=4), :]),
                      lambda k: sel(wu[1, k, pl.ds(p0, 8, stride=4), :]))
            return carry

        jax.lax.fori_loop(0, 8, mid, 0)
    mid_group(512,
              lambda k: jnp.broadcast_to(wny[0, :, 128 * k:128 * (k + 1)].astype(f32), (8, 128)),
              lambda k: jnp.broadcast_to(wny[1, :, 128 * k:128 * (k + 1)].astype(f32), (8, 128)))

    def inv(i, carry):
        @pl.when(i == WO_AT)
        def _():
            start(c_o)

        ys = []
        for half in range(2):
            n1 = 2 * i + half
            c0 = pl.multiple_of(n1 * 128, 128)
            mm = pltpu.bitcast(ms[n1], bf16)
            zc = jnp.concatenate([tr[0:512, pl.ds(c0, 128)], ti[0:512, pl.ds(c0, 128)]], axis=1)
            z = _dot_nt(mm, zc)
            zn = jnp.concatenate([tr[512:640, pl.ds(c0, 128)], ti[512:640, pl.ds(c0, 128)]], axis=1)
            ny = _dot_nt(mm[0:128], zn)
            zr, zi = z[0:128], z[128:256]
            zi0 = jnp.where(lane == 0, ny, zi[:, 0:128])
            u = _dot(jnp.concatenate([zr[:, 0:128], zi0], axis=1), cmat(_C_G))
            v = [_dot(jnp.concatenate([zr[:, 128 * j:128 * (j + 1)], zi[:, 128 * j:128 * (j + 1)]], axis=1),
                      cmat(_C_G + j)) for j in (1, 2, 3)]
            u0, u4 = u[:, 0:128], u[:, 128:256]
            v1r, v1i = v[0][:, 0:128], v[0][:, 128:256]
            v2r, v2i = v[1][:, 0:128], v[1][:, 128:256]
            v3r, v3i = v[2][:, 0:128], v[2][:, 128:256]
            e, o = u0 + u4, u0 - u4
            ep, em = e + v2r, e - v2r
            sa, da = v1r + v3r, v1r - v3r
            di, si = v1i - v3i, v1i + v3i
            p, q = (da - si) * _R2, (da + si) * _R2
            om, op = o - v2i, o + v2i
            ys.append([ep + sa, om + p, em - di, op - q, ep - sa, om - p, em + di, op + q])
        for a in range(8):
            bu[a, pl.ds(i, 128, stride=8), :] = (_bf16_word(ys[0][a]) >> 16) | _bf16_word(ys[1][a])
        return carry

    jax.lax.fori_loop(0, 8, inv, 0)

    wait(c_p)
    h_ref[0, 0:M, :] = mem0_ref[...].astype(f32)
    row = jax.lax.broadcasted_iota(i32, (L, L), 0)
    col = jax.lax.broadcasted_iota(i32, (L, L), 1)
    mask = (row < M) | (row >= col)
    scale = DH ** -0.5

    def load_x(s, hb):
        p0 = s * (SEG // 2) if isinstance(s, int) else pl.multiple_of(s * (SEG // 2), SEG // 2)
        for a in range(8):
            h_ref[hb, M:L, 128 * a:128 * (a + 1)] = pltpu.bitcast(xu[a, pl.ds(p0, SEG // 2), :], bf16).astype(f32)

    def probs(sc):
        sc = jnp.where(mask, sc * scale, -1e9)
        e = jnp.exp(sc - jnp.max(sc, axis=-1, keepdims=True))
        return e * (1.0 / jnp.sum(e, axis=-1, keepdims=True))

    def gate(hb):
        gw = gw_ref[...].astype(f32).reshape(1, D)
        return jax.nn.sigmoid(jnp.sum(h_ref[hb, M:L, :] * gw, axis=-1, keepdims=True))

    def finish(s, hn, j, r, g):
        r0 = s * SEG if isinstance(s, int) else pl.multiple_of(s * SEG, SEG)
        p0 = s * (SEG // 2) if isinstance(s, int) else pl.multiple_of(s * (SEG // 2), SEG // 2)
        c0 = j * 128
        h_ref[hn, 0:M, pl.ds(c0, 128)] = r[0:M]
        bb = pltpu.bitcast(bu[j, pl.ds(p0, SEG // 2), :], bf16).astype(f32)
        ob[pl.ds(r0, SEG), pl.ds(c0, 128)] = (bb + g * (r[M:L] - bb)).astype(bf16)

    def out_copy(s):
        r0 = s * SEG if isinstance(s, int) else pl.multiple_of(s * SEG, SEG)
        return pltpu.make_async_copy(ob.at[pl.ds(r0, SEG)], out_hbm.at[pl.ds(r0, SEG)], osem)

    def repack(i, carry):
        for t, w in enumerate((wq_hbm, wk_hbm, wv_hbm)):
            pltpu.make_async_copy(w.bitcast(u32).at[:, i, :], wraw.at[t, i], qsem.at[i]).wait()
        for t in range(3):
            ev = wraw[t, i, pl.ds(0, 512, stride=2), :]
            od = wraw[t, i, pl.ds(1, 512, stride=2), :]
            wqkv[2 * i, :, 128 * t:128 * (t + 1)] = (ev & jnp.uint32(0xFFFF)) | (od << 16)
            wqkv[2 * i + 1, :, 128 * t:128 * (t + 1)] = (ev >> 16) | (od & jnp.uint32(0xFFFF0000))
        return carry

    jax.lax.fori_loop(0, 16, repack, 0)
    load_x(0, 0)


    def step(s, hb, first):
        hn = (hb + 1) % UNROLL
        st = {}

        def qk(a):
            qkv = st[a]['qkv']
            st[a]['sc'] = _dot_nt(qkv[:, 0:128], qkv[:, 128:256])

        def softmax(a):
            st[a]['p'] = probs(st[a]['sc'])

        def pv(b):
            o_ref[:, b * 128:(b + 1) * 128] = _dot(st[b]['p'], st[b]['qkv'][:, 256:384])
            del st[b]

        for it in range(H):
            if it == 0:
                r = _dot(h_ref[hb, :, 0:512], pltpu.bitcast(wqkv[it, 0:256], bf16))
                st[it] = dict(qkv=_dot(h_ref[hb, :, 512:1024], pltpu.bitcast(wqkv[it, 256:512], bf16)) + r)
            else:
                st[it] = dict(qkv=_dot(h_ref[hb], pltpu.bitcast(wqkv[it], bf16)))
            if it >= LAGQ:
                qk(it - LAGQ)
            if it >= LAGP:
                pv(it - LAGP)
            if it >= LAGQ:
                softmax(it - LAGQ)
            if it == XAT:
                g = gate(hb)
                load_x(min(s + 1, NSEG - 1) if isinstance(s, int) else jnp.minimum(s + 1, NSEG - 1), hn)

        def wo_dot(j, h0, h1):
            w = wo2[j // 4, h0:h1, :, 128 * (j % 4):128 * (j % 4 + 1)]
            return _dot(o_ref[:, h0 * DH:h1 * DH], pltpu.bitcast(w.reshape((h1 - h0) * 64, 128), bf16))

        if first:
            for a in range(H - LAGQ, H):
                qk(a)
                softmax(a)
            for b in range(H - LAGP, H):
                pv(b)
            for hf in range(2):
                for q in range(4):
                    c_o[4 * hf + q].wait()
                    for j in range(4 * hf, 4 * hf + 4):
                        r = wo_dot(j, 8 * q, 8 * q + 8)
                        if q > 0:
                            r = part_ref[:, 128 * j:128 * (j + 1)] + r
                        if q < 3:
                            part_ref[:, 128 * j:128 * (j + 1)] = r
                        else:
                            finish(s, hn, j, r, g)
        else:
            tail = []
            for t in range(LAGP):
                fns = []
                if t < LAGQ:
                    fns.append(lambda a=H - LAGQ + t: qk(a))
                if t < LAGP - 1:
                    fns.append(lambda b=H - LAGP + t: pv(b))
                if t < LAGQ:
                    fns.append(lambda a=H - LAGQ + t: softmax(a))
                tail.append(fns)
            tail = tail[:max(LAGQ, LAGP - 1)] + [[], [lambda: pv(H - 1)]]
            npart = len(tail)
            order = list(range(8 - npart, 8))
            for t, j in enumerate(order):
                part_ref[:, 128 * t:128 * (t + 1)] = wo_dot(j, 0, KS)
                for fn in tail[t]:
                    fn()
            for j in range(8 - npart):
                finish(s, hn, j, wo_dot(j, 0, H), g)
            for t, j in enumerate(order):
                finish(s, hn, j, part_ref[:, 128 * t:128 * (t + 1)] + wo_dot(j, KS, H), g)
        out_copy(s).start()

    assert (NSEG - 1) % UNROLL == 0
    step(0, 0, True)

    def next_step(t, carry):
        for u in range(UNROLL):
            step(1 + t * UNROLL + u, (1 + u) % UNROLL, False)
        return carry

    jax.lax.fori_loop(0, (NSEG - 1) // UNROLL, next_step, 0)

    pltpu.make_async_copy(ob, out_hbm, osem).wait()


@functools.partial(jax.jit, static_argnames=("A_seg_len",))
def pallas_gated_mix__memory_aug_recurrent_mem_tr__spectral_gfnet__prompt_kernel(
    A_x, A_mem0, A_Wq, A_Wk, A_Wv, A_Wo, A_seg_len, B_x, B_w_r, B_w_i, gate_w,
):
    del B_x
    assert A_x.shape == (1, S, D) and A_mem0.shape == (1, M, D) and A_Wq.shape == (D, H, DH)
    assert int(A_seg_len) == SEG
    V = pltpu.VMEM
    hbm = pl.BlockSpec(memory_space=pltpu.MemorySpace.HBM)
    vm = pl.BlockSpec(memory_space=pltpu.MemorySpace.VMEM)
    out = pl.pallas_call(
        _kernel,
        out_shape=jax.ShapeDtypeStruct((S, D), bf16),
        in_specs=[hbm] * 9,
        out_specs=hbm,
        scratch_shapes=[
            V((M, D), bf16),
            V((D,), bf16),
            V((8, S // 2, 128), u32),
            V((3, 16, D, 128), u32),
            V((H, D // 2, 384), u32),
            V((2, H, DH // 2, 512), u32),
            V((7, 128, 256), u32),
            V((520, 128), f32),
            V((16, 128, 256), u32),
            V((2, 16, 256, 128), u32),
            V((2, 1, S), bf16),
            V((640, S), f32),
            V((640, S), f32),
            V((8, S // 2, 128), u32),
            V((UNROLL, L, D), f32),
            V((L, H * DH), f32),
            V((L, D), f32),
            V((S, D), bf16),
            pltpu.SemaphoreType.DMA((3,)),
            pltpu.SemaphoreType.DMA((16,)),
            pltpu.SemaphoreType.DMA((8,)),
            pltpu.SemaphoreType.DMA,
        ],
        compiler_params=pltpu.CompilerParams(vmem_limit_bytes=112 * 1024 * 1024),
    )(A_x.reshape(S, D), A_mem0.reshape(M, D), A_Wq, A_Wk, A_Wv, A_Wo,
      B_w_r.T, B_w_i.T, gate_w)
    return out.reshape(1, S, D)
```

```python
import functools

import jax
import jax.numpy as jnp
import numpy as np
import jax.experimental.pallas as pl
import jax.experimental.pallas.tpu as pltpu

f32 = jnp.float32
bf16 = jnp.bfloat16
u32 = jnp.uint32
i32 = jnp.int32

S, D, H, DH, M, SEG = 2048, 1024, 32, 128, 8, 32
L = M + SEG
NSEG = S // SEG
WO_AT = 5
UNROLL = 3
LAGQ, LAGP = 1, 3
KS = 28
XAT = 8
KR = 520


_C_A, _C_G = 0, 3


def _dot(a, b):
    return jax.lax.dot_general(a, b, (((1,), (0,)), ((), ())), preferred_element_type=f32)


def _dot_nt(a, b):
    return jax.lax.dot_general(a, b, (((1,), (1,)), ((), ())), preferred_element_type=f32)


def _lo(w):
    return pltpu.bitcast(w << 16, f32)


def _hi(w):
    return pltpu.bitcast(w & np.uint32(0xFFFF0000), f32)


def _bf16_word(x):
    return pltpu.bitcast(x.astype(bf16).astype(f32), u32)


_R2 = float(np.sqrt(0.5))


def _cmul_const(z, ang):
    zr, zi = z
    c, s = float(np.cos(ang)), float(np.sin(ang))
    q = int(round(ang / (np.pi / 4)))
    if abs(ang - q * np.pi / 4) < 1e-9:
        q %= 8
        if q == 0:
            return zr, zi
        if q == 2:
            return -zi, zr
        if q == 4:
            return -zr, -zi
        if q == 6:
            return zi, -zr
        if q == 1:
            return (zr - zi) * _R2, (zr + zi) * _R2
        if q == 3:
            return (zr + zi) * (-_R2), (zr - zi) * _R2
        if q == 5:
            return (zi - zr) * _R2, (zr + zi) * (-_R2)
        return (zr + zi) * _R2, (zi - zr) * _R2
    return zr * c - zi * s, zr * s + zi * c


def _add(a, b):
    return a[0] + b[0], a[1] + b[1]


def _sub(a, b):
    return a[0] - b[0], a[1] - b[1]


def _bfly4(x0, x1, x2, x3, sign):
    s0, s1 = _add(x0, x2), _sub(x0, x2)
    s2, s3 = _add(x1, x3), _sub(x1, x3)
    y0, y2 = _add(s0, s2), _sub(s0, s2)
    if sign < 0:
        y1 = (s1[0] + s3[1], s1[1] - s3[0])
        y3 = (s1[0] - s3[1], s1[1] + s3[0])
    else:
        y1 = (s1[0] - s3[1], s1[1] + s3[0])
        y3 = (s1[0] + s3[1], s1[1] - s3[0])
    return y0, y1, y2, y3


def _fft16(x, sign):
    t = [[None] * 4 for _ in range(4)]
    for b in range(4):
        y = _bfly4(x[b], x[4 + b], x[8 + b], x[12 + b], sign)
        for c in range(4):
            t[c][b] = _cmul_const(y[c], sign * 2 * np.pi * b * c / 16)
    out = [None] * 16
    for c in range(4):
        y = _bfly4(t[c][0], t[c][1], t[c][2], t[c][3], sign)
        for d in range(4):
            out[c + 4 * d] = y[d]
    return out


def _kernel(x_hbm, mem0_hbm, wq_hbm, wk_hbm, wv_hbm, wo_hbm, wrt_hbm, wit_hbm, gw_hbm,
            out_hbm,
            mem0_ref, gw_ref, xu, wraw, wqkv, wo2, cu, ca, ms, wu, wny, tr, ti, bu, h_ref, o_ref, part_ref, ob, sems, qsem, wsem, osem):
    def start(cs):
        for c in cs:
            c.start()

    def wait(cs):
        for c in cs:
            c.wait()

    c_x = [pltpu.make_async_copy(x_hbm, ob, sems.at[0])]
    c_w = []
    for t, w in enumerate((wrt_hbm, wit_hbm)):
        ww = w.at[0:512].bitcast(u32)
        c_w += [pltpu.make_async_copy(ww.at[:, 128 * k:128 * (k + 1)], wu.at[t, k, 0:256], sems.at[1]) for k in range(16)]
        c_w.append(pltpu.make_async_copy(w.at[512:513], wny.at[t], sems.at[1]))
    c_qkv = [[pltpu.make_async_copy(w.bitcast(u32).at[:, i, :], wraw.at[t, i, 0:D], qsem.at[i])
              for t, w in enumerate((wq_hbm, wk_hbm, wv_hbm))] for i in range(16)]
    wow = wo_hbm.bitcast(u32)
    c_o = [pltpu.make_async_copy(wow.at[8 * q:8 * q + 8, :, 512 * hf:512 * (hf + 1)], wo2.at[hf, 8 * q:8 * q + 8],
                                 wsem.at[4 * hf + q]) for hf in range(2) for q in range(4)]
    c_p = [pltpu.make_async_copy(mem0_hbm, mem0_ref, sems.at[2]), pltpu.make_async_copy(gw_hbm, gw_ref, sems.at[2])]
    start(c_x)
    start(c_p)
    start(c_w)

    lane = jax.lax.broadcasted_iota(i32, (128, 128), 1)

    def cmat(i):
        return pltpu.bitcast(cu[i], bf16)

    rowi = jax.lax.broadcasted_iota(i32, (128, 128), 0)
    first = rowi < 64
    gscale = 1.0 / (D * S)

    def pack(m):
        return pltpu.bitcast(m.astype(bf16), u32)

    def blk2(a, b, c, d):
        return jnp.concatenate([jnp.concatenate([a, b], axis=1), jnp.concatenate([c, d], axis=1)], axis=0)

    alt = jnp.where((lane & 1) == 0, 1.0, -1.0).astype(f32)
    for j in range(4):
        lo, hi = (0, 4) if j == 0 else (j, 8 - j)
        k = jnp.where(first, lo + 8 * rowi, hi + 8 * (rowi - 64))
        ang = ((k * lane) & (D - 1)).astype(f32) * (2 * np.pi / D)
        c, s = jnp.cos(ang), jnp.sin(ang)
        if j == 0:
            ca[0:64, :] = c[0:64]
            ca[64:128, :] = -s[0:64]
            ca[128:136, :] = jnp.where(rowi[0:8] == 0, alt[0:8], 0.0)
            ca[136:200, :] = c[64:128]
            ca[200:264, :] = -s[64:128]
            c2 = jnp.where(rowi == 0, c, 2.0 * c) * gscale
            s2 = jnp.where(rowi == 0, alt, -2.0 * s) * gscale
            cu[_C_G] = pack(blk2(jnp.where(first, c2, 0.0), jnp.where(first, 0.0, c2),
                                 jnp.where(first, s2, 0.0), jnp.where(first, 0.0, s2)))
        else:
            sg = jnp.where(first, -s, s)
            cg = jnp.where(first, -c, c)
            cu[_C_A + j - 1] = pack(blk2(c, sg, -s, cg))
            cu[_C_G + j] = pack(blk2(2.0 * gscale * c, -2.0 * gscale * sg, -2.0 * gscale * s, -2.0 * gscale * cg))
    ang = ((rowi * lane) & 127).astype(f32) * (2 * np.pi / 128)
    ca[264:392, :] = jnp.cos(ang)
    ca[392:520, :] = -jnp.sin(ang)
    tr[KR:, :] = jnp.zeros((640 - KR, S), f32)
    ti[KR:, :] = jnp.zeros((640 - KR, S), f32)

    def gen_ms(n1, carry):
        fr, fi = ca[264:392, :], ca[392:520, :]
        ang = (n1 * lane[0:8]).astype(f32) * (2 * np.pi / S)
        t_r = jnp.broadcast_to(jnp.cos(ang)[0:1], (128, 128))
        t_i = jnp.broadcast_to(-jnp.sin(ang)[0:1], (128, 128))
        mr, mi = fr * t_r - fi * t_i, fr * t_i + fi * t_r
        ms[n1] = pack(blk2(mr, mi, -mi, mr))
        return carry

    jax.lax.fori_loop(0, 16, gen_ms, 0)
    wait(c_x)
    for c in c_qkv:
        start(c)

    def split_x(c, carry):
        r0 = pl.multiple_of(c * 128, 128)
        for a in range(8):
            xu[a, pl.ds(pl.multiple_of(c * 64, 64), 64), :] = pltpu.bitcast(ob[pl.ds(r0, 128), 128 * a:128 * (a + 1)], u32)
        return carry

    jax.lax.fori_loop(0, 16, split_x, 0)

    def fwd(i, carry):
        xw_t = [xu[a, pl.ds(i, 128, stride=8), :] for a in range(8)]
        for half in range(2):
            n1 = 2 * i + half
            x = [(_lo if half == 0 else _hi)(w) for w in xw_t]
            a0, a1, a2, a3 = x[0] + x[4], x[1] + x[5], x[2] + x[6], x[3] + x[7]
            d0, d1, d2, d3 = x[0] - x[4], x[1] - x[5], x[2] - x[6], x[3] - x[7]
            e0, e1 = a0 + a2, a1 + a3
            u, w = (d1 - d3) * _R2, (d1 + d3) * _R2
            p0, p4 = e0 + e1, e0 - e1
            planes = [(d0 + u, d2 + w), (a0 - a2, a1 - a3), (d0 - u, w - d2)]
            o0 = _dot_nt(ca[0:136, :], p0)
            o4 = _dot_nt(ca[136:264, :], p4)
            oj = [_dot_nt(cmat(_C_A + j), jnp.concatenate(planes[j], axis=1)) for j in range(3)]
            xr = jnp.concatenate([o0[0:64], o4[0:64]] + [o[0:128] for o in oj] + [o0[128:136]], axis=0)
            xi = jnp.concatenate([o0[64:128], o4[64:128]] + [o[128:256] for o in oj]
                                 + [jnp.zeros((8, 128), f32)], axis=0)
            t = _dot(jnp.concatenate([xr, xi], axis=1), pltpu.bitcast(ms[n1], bf16))
            c0 = pl.multiple_of(n1 * 128, 128)
            tr[0:KR, pl.ds(c0, 128)] = t[:, 0:128]
            ti[0:KR, pl.ds(c0, 128)] = t[:, 128:256]
        return carry

    jax.lax.fori_loop(0, 8, fwd, 0)

    wait(c_w)

    def mid_group(r0, wr_fn, wi_fn):
        z = [(tr[pl.ds(r0, 8), 128 * n:128 * (n + 1)], ti[pl.ds(r0, 8), 128 * n:128 * (n + 1)]) for n in range(16)]
        z = _fft16(z, -1)
        q = []
        for k in range(16):
            wr, wi = wr_fn(k), wi_fn(k)
            zr, zi = z[k]
            q.append((zr * wr - zi * wi, zr * wi + zi * wr))
        z = _fft16(q, +1)
        for n in range(16):
            tr[pl.ds(r0, 8), 128 * n:128 * (n + 1)] = z[n][0]
            ti[pl.ds(r0, 8), 128 * n:128 * (n + 1)] = z[n][1]

    for blk, half, res in ((0, 0, 0), (0, 1, 4), (1, 0, 1), (1, 1, 7), (2, 0, 2), (2, 1, 6), (3, 0, 3), (3, 1, 5)):
        sel = _lo if res % 2 == 0 else _hi

        def mid(g, carry, blk=blk, half=half, res=res, sel=sel):
            r0 = pl.multiple_of(128 * blk + 64 * half + 8 * g, 8)
            p0 = res // 2 + 32 * g
            mid_group(r0,
                      lambda k: sel(wu[0, k, pl.ds(p0, 8, stride=4), :]),
                      lambda k: sel(wu[1, k, pl.ds(p0, 8, stride=4), :]))
            return carry

        jax.lax.fori_loop(0, 8, mid, 0)
    mid_group(512,
              lambda k: jnp.broadcast_to(wny[0, :, 128 * k:128 * (k + 1)].astype(f32), (8, 128)),
              lambda k: jnp.broadcast_to(wny[1, :, 128 * k:128 * (k + 1)].astype(f32), (8, 128)))

    def inv(i, carry):
        @pl.when(i == WO_AT)
        def _():
            start(c_o)

        ys = []
        for half in range(2):
            n1 = 2 * i + half
            c0 = pl.multiple_of(n1 * 128, 128)
            mm = pltpu.bitcast(ms[n1], bf16)
            zc = jnp.concatenate([tr[0:512, pl.ds(c0, 128)], ti[0:512, pl.ds(c0, 128)]], axis=1)
            z = _dot_nt(mm, zc)
            zn = jnp.concatenate([tr[512:640, pl.ds(c0, 128)], ti[512:640, pl.ds(c0, 128)]], axis=1)
            ny = _dot_nt(mm[0:128], zn)
            zr, zi = z[0:128], z[128:256]
            zi0 = jnp.where(lane == 0, ny, zi[:, 0:128])
            u = _dot(jnp.concatenate([zr[:, 0:128], zi0], axis=1), cmat(_C_G))
            v = [_dot(jnp.concatenate([zr[:, 128 * j:128 * (j + 1)], zi[:, 128 * j:128 * (j + 1)]], axis=1),
                      cmat(_C_G + j)) for j in (1, 2, 3)]
            u0, u4 = u[:, 0:128], u[:, 128:256]
            v1r, v1i = v[0][:, 0:128], v[0][:, 128:256]
            v2r, v2i = v[1][:, 0:128], v[1][:, 128:256]
            v3r, v3i = v[2][:, 0:128], v[2][:, 128:256]
            e, o = u0 + u4, u0 - u4
            ep, em = e + v2r, e - v2r
            sa, da = v1r + v3r, v1r - v3r
            di, si = v1i - v3i, v1i + v3i
            p, q = (da - si) * _R2, (da + si) * _R2
            om, op = o - v2i, o + v2i
            ys.append([ep + sa, om + p, em - di, op - q, ep - sa, om - p, em + di, op + q])
        for a in range(8):
            bu[a, pl.ds(i, 128, stride=8), :] = (_bf16_word(ys[0][a]) >> 16) | _bf16_word(ys[1][a])
        return carry

    jax.lax.fori_loop(0, 8, inv, 0)

    wait(c_p)
    h_ref[0, 0:M, :] = mem0_ref[...].astype(f32)
    row = jax.lax.broadcasted_iota(i32, (L, L), 0)
    col = jax.lax.broadcasted_iota(i32, (L, L), 1)
    mask = (row < M) | (row >= col)
    scale = DH ** -0.5

    def load_x(s, hb):
        p0 = s * (SEG // 2) if isinstance(s, int) else pl.multiple_of(s * (SEG // 2), SEG // 2)
        for a in range(8):
            h_ref[hb, M:L, 128 * a:128 * (a + 1)] = pltpu.bitcast(xu[a, pl.ds(p0, SEG // 2), :], bf16).astype(f32)

    def probs(sc):
        sc = jnp.where(mask, sc * scale, -1e9)
        e = jnp.exp(sc - jnp.max(sc, axis=-1, keepdims=True))
        return e * (1.0 / jnp.sum(e, axis=-1, keepdims=True))

    def gate(hb):
        gw = gw_ref[...].astype(f32).reshape(1, D)
        return jax.nn.sigmoid(jnp.sum(h_ref[hb, M:L, :] * gw, axis=-1, keepdims=True))

    def finish(s, hn, j, r, g):
        r0 = s * SEG if isinstance(s, int) else pl.multiple_of(s * SEG, SEG)
        p0 = s * (SEG // 2) if isinstance(s, int) else pl.multiple_of(s * (SEG // 2), SEG // 2)
        c0 = j * 128
        h_ref[hn, 0:M, pl.ds(c0, 128)] = r[0:M]
        bb = pltpu.bitcast(bu[j, pl.ds(p0, SEG // 2), :], bf16).astype(f32)
        ob[pl.ds(r0, SEG), pl.ds(c0, 128)] = (bb + g * (r[M:L] - bb)).astype(bf16)

    def out_copy(s):
        r0 = s * SEG if isinstance(s, int) else pl.multiple_of(s * SEG, SEG)
        return pltpu.make_async_copy(ob.at[pl.ds(r0, SEG)], out_hbm.at[pl.ds(r0, SEG)], osem)

    def repack(i, carry):
        for t, w in enumerate((wq_hbm, wk_hbm, wv_hbm)):
            pltpu.make_async_copy(w.bitcast(u32).at[:, i, :], wraw.at[t, i, 0:D], qsem.at[i]).wait()
        for t in range(3):
            ev = wraw[t, i, pl.ds(0, 512, stride=2), :]
            od = wraw[t, i, pl.ds(1, 512, stride=2), :]
            wqkv[2 * i, :, 128 * t:128 * (t + 1)] = (ev & np.uint32(0xFFFF)) | (od << 16)
            wqkv[2 * i + 1, :, 128 * t:128 * (t + 1)] = (ev >> 16) | (od & np.uint32(0xFFFF0000))
        return carry

    jax.lax.fori_loop(0, 16, repack, 0)
    load_x(0, 0)


    def step(s, hb, first):
        hn = (hb + 1) % UNROLL
        st = {}

        def qk(a):
            qkv = st[a]['qkv']
            st[a]['sc'] = _dot_nt(qkv[:, 0:128], qkv[:, 128:256])

        def softmax(a):
            st[a]['p'] = probs(st[a]['sc'])

        def pv(b):
            o_ref[:, b * 128:(b + 1) * 128] = _dot(st[b]['p'], st[b]['qkv'][:, 256:384])
            del st[b]

        for it in range(H):
            if it == 0:
                r = _dot(h_ref[hb, :, 0:512], pltpu.bitcast(wqkv[it, 0:256], bf16))
                st[it] = dict(qkv=_dot(h_ref[hb, :, 512:1024], pltpu.bitcast(wqkv[it, 256:512], bf16)) + r)
            else:
                st[it] = dict(qkv=_dot(h_ref[hb], pltpu.bitcast(wqkv[it], bf16)))
            if it >= LAGQ:
                qk(it - LAGQ)
            if it >= LAGP:
                pv(it - LAGP)
            if it >= LAGQ:
                softmax(it - LAGQ)
            if it == XAT:
                g = gate(hb)
                load_x(min(s + 1, NSEG - 1) if isinstance(s, int) else jnp.minimum(s + 1, NSEG - 1), hn)

        def wo_dot(j, h0, h1):
            w = wo2[j // 4, h0:h1, :, 128 * (j % 4):128 * (j % 4 + 1)]
            return _dot(o_ref[:, h0 * DH:h1 * DH], pltpu.bitcast(w.reshape((h1 - h0) * 64, 128), bf16))

        if first:
            for a in range(H - LAGQ, H):
                qk(a)
                softmax(a)
            for b in range(H - LAGP, H):
                pv(b)
            for hf in range(2):
                for q in range(4):
                    c_o[4 * hf + q].wait()
                    for j in range(4 * hf, 4 * hf + 4):
                        r = wo_dot(j, 8 * q, 8 * q + 8)
                        if q > 0:
                            r = part_ref[:, 128 * j:128 * (j + 1)] + r
                        if q < 3:
                            part_ref[:, 128 * j:128 * (j + 1)] = r
                        else:
                            finish(s, hn, j, r, g)
        else:
            tail = []
            for t in range(LAGP):
                fns = []
                if t < LAGQ:
                    fns.append(lambda a=H - LAGQ + t: qk(a))
                if t < LAGP - 1:
                    fns.append(lambda b=H - LAGP + t: pv(b))
                if t < LAGQ:
                    fns.append(lambda a=H - LAGQ + t: softmax(a))
                tail.append(fns)
            tail = tail[:max(LAGQ, LAGP - 1)] + [[], [lambda: pv(H - 1)]]
            npart = len(tail)
            order = list(range(8 - npart, 8))
            for t, j in enumerate(order):
                part_ref[:, 128 * t:128 * (t + 1)] = wo_dot(j, 0, KS)
                for fn in tail[t]:
                    fn()
            for j in range(8 - npart):
                finish(s, hn, j, wo_dot(j, 0, H), g)
            for t, j in enumerate(order):
                finish(s, hn, j, part_ref[:, 128 * t:128 * (t + 1)] + wo_dot(j, KS, H), g)
        out_copy(s).start()

    assert (NSEG - 1) % UNROLL == 0
    step(0, 0, True)

    def next_step(t, carry):
        for u in range(UNROLL):
            step(1 + t * UNROLL + u, (1 + u) % UNROLL, False)
        return carry

    jax.lax.fori_loop(0, (NSEG - 1) // UNROLL, next_step, 0)

    pltpu.make_async_copy(ob, out_hbm, osem).wait()


@functools.partial(jax.jit, static_argnames=("A_seg_len",))
def pallas_gated_mix__memory_aug_recurrent_mem_tr__spectral_gfnet__prompt_kernel(
    A_x, A_mem0, A_Wq, A_Wk, A_Wv, A_Wo, A_seg_len, B_x, B_w_r, B_w_i, gate_w,
):
    del B_x
    assert A_x.shape == (1, S, D) and A_mem0.shape == (1, M, D) and A_Wq.shape == (D, H, DH)
    assert int(A_seg_len) == SEG
    V = pltpu.VMEM
    hbm = pl.BlockSpec(memory_space=pltpu.MemorySpace.HBM)
    vm = pl.BlockSpec(memory_space=pltpu.MemorySpace.VMEM)
    out = pl.pallas_call(
        _kernel,
        out_shape=jax.ShapeDtypeStruct((S, D), bf16),
        in_specs=[hbm] * 9,
        out_specs=hbm,
        scratch_shapes=[
            V((M, D), bf16),
            V((D,), bf16),
            V((8, S // 2 + 8, 128), u32),
            V((3, 16, D + 8, 128), u32),
            V((H, D // 2, 384), u32),
            V((2, H, DH // 2, 512), u32),
            V((7, 128, 256), u32),
            V((520, 128), f32),
            V((16, 128, 256), u32),
            V((2, 16, 256 + 8, 128), u32),
            V((2, 1, S), bf16),
            V((640, S), f32),
            V((640, S), f32),
            V((8, S // 2 + 8, 128), u32),
            V((UNROLL, L, D), f32),
            V((L, H * DH), f32),
            V((L, D), f32),
            V((S, D), bf16),
            pltpu.SemaphoreType.DMA((3,)),
            pltpu.SemaphoreType.DMA((16,)),
            pltpu.SemaphoreType.DMA((8,)),
            pltpu.SemaphoreType.DMA,
        ],
        compiler_params=pltpu.CompilerParams(vmem_limit_bytes=112 * 1024 * 1024),
    )(A_x.reshape(S, D), A_mem0.reshape(M, D), A_Wq, A_Wk, A_Wv, A_Wo,
      B_w_r.T, B_w_i.T, gate_w)
    return out.reshape(1, S, D)
```

```python
import functools

import jax
import jax.numpy as jnp
import numpy as np
import jax.experimental.pallas as pl
import jax.experimental.pallas.tpu as pltpu

f32 = jnp.float32
bf16 = jnp.bfloat16
u32 = jnp.uint32
i32 = jnp.int32

S, D, H, DH, M, SEG = 2048, 1024, 32, 128, 8, 32
L = M + SEG
NSEG = S // SEG
UNROLL = 3
LAGQ, LAGP = 1, 3
KS = 28
XAT = 8
KR = 520
_C_A, _C_G = 0, 3


def _dot(a, b):
    return jax.lax.dot_general(a, b, (((1,), (0,)), ((), ())), preferred_element_type=f32)


def _dot_nt(a, b):
    return jax.lax.dot_general(a, b, (((1,), (1,)), ((), ())), preferred_element_type=f32)


def _lo(w):
    return pltpu.bitcast(w << 16, f32)


def _hi(w):
    return pltpu.bitcast(w & np.uint32(0xFFFF0000), f32)


def _bf16_word(x):
    return pltpu.bitcast(x.astype(bf16).astype(f32), u32)


_R2 = float(np.sqrt(0.5))


def _cmul_const(z, ang):
    zr, zi = z
    c, s = float(np.cos(ang)), float(np.sin(ang))
    q = int(round(ang / (np.pi / 4)))
    if abs(ang - q * np.pi / 4) < 1e-9:
        q %= 8
        if q == 0:
            return zr, zi
        if q == 2:
            return -zi, zr
        if q == 4:
            return -zr, -zi
        if q == 6:
            return zi, -zr
        if q == 1:
            return (zr - zi) * _R2, (zr + zi) * _R2
        if q == 3:
            return (zr + zi) * (-_R2), (zr - zi) * _R2
        if q == 5:
            return (zi - zr) * _R2, (zr + zi) * (-_R2)
        return (zr + zi) * _R2, (zi - zr) * _R2
    return zr * c - zi * s, zr * s + zi * c


def _add(a, b):
    return a[0] + b[0], a[1] + b[1]


def _sub(a, b):
    return a[0] - b[0], a[1] - b[1]


def _bfly4(x0, x1, x2, x3, sign):
    s0, s1 = _add(x0, x2), _sub(x0, x2)
    s2, s3 = _add(x1, x3), _sub(x1, x3)
    y0, y2 = _add(s0, s2), _sub(s0, s2)
    if sign < 0:
        y1 = (s1[0] + s3[1], s1[1] - s3[0])
        y3 = (s1[0] - s3[1], s1[1] + s3[0])
    else:
        y1 = (s1[0] - s3[1], s1[1] + s3[0])
        y3 = (s1[0] + s3[1], s1[1] - s3[0])
    return y0, y1, y2, y3


def _fft16(x, sign):
    t = [[None] * 4 for _ in range(4)]
    for b in range(4):
        y = _bfly4(x[b], x[4 + b], x[8 + b], x[12 + b], sign)
        for c in range(4):
            t[c][b] = _cmul_const(y[c], sign * 2 * np.pi * b * c / 16)
    out = [None] * 16
    for c in range(4):
        y = _bfly4(t[c][0], t[c][1], t[c][2], t[c][3], sign)
        for d in range(4):
            out[c + 4 * d] = y[d]
    return out


def _kernel(x_hbm, mem0_hbm, wq_hbm, wk_hbm, wv_hbm, wo_hbm, wrt_hbm, wit_hbm, gw_hbm,
            out_hbm,
            mem0_ref, gw_ref, xu, wraw, wqkv, wo2, cu, ca, ms, wu, wny, tr, ti, bu, h_ref, o_ref, part_ref, xq_ref, wsp_ref, ob, sems, qsem, wsem, osem):
    def start(cs):
        for c in cs:
            c.start()

    def wait(cs):
        for c in cs:
            c.wait()

    c_x = [pltpu.make_async_copy(x_hbm.at[1024 * c:1024 * c + 1024], ob.at[1024 * c:1024 * c + 1024], sems.at[3 * c])
           for c in range(2)]
    c_w = []
    for t, w in enumerate((wrt_hbm, wit_hbm)):
        ww = w.at[0:512].bitcast(u32)
        c_w += [pltpu.make_async_copy(ww.at[:, 128 * k:128 * (k + 1)], wu.at[t, k, 0:256], sems.at[1]) for k in range(16)]
        c_w.append(pltpu.make_async_copy(w.at[512:513], wny.at[t], sems.at[1]))
    wow = wo_hbm.bitcast(u32)
    c_o = [pltpu.make_async_copy(wow.at[8 * q:8 * q + 8, :, 512 * hf:512 * (hf + 1)], wo2.at[hf, 8 * q:8 * q + 8],
                                 wsem.at[4 * hf + q]) for hf in (1, 0) for q in range(4)]
    c_p = [pltpu.make_async_copy(mem0_hbm, mem0_ref, sems.at[2]), pltpu.make_async_copy(gw_hbm, gw_ref, sems.at[2])]
    start(c_x)
    start(c_p)
    start(c_w)

    lane = jax.lax.broadcasted_iota(i32, (128, 128), 1)

    def cmat(i):
        return pltpu.bitcast(cu[i], bf16)

    rowi = jax.lax.broadcasted_iota(i32, (128, 128), 0)
    first = rowi < 64
    gscale = 1.0 / (D * S)

    def pack(m):
        return pltpu.bitcast(m.astype(bf16), u32)

    def blk2(a, b, c, d):
        return jnp.concatenate([jnp.concatenate([a, b], axis=1), jnp.concatenate([c, d], axis=1)], axis=0)

    alt = jnp.where((lane & 1) == 0, 1.0, -1.0).astype(f32)
    for j in range(4):
        lo, hi = (0, 4) if j == 0 else (j, 8 - j)
        k = jnp.where(first, lo + 8 * rowi, hi + 8 * (rowi - 64))
        ang = ((k * lane) & (D - 1)).astype(f32) * (2 * np.pi / D)
        c, s = jnp.cos(ang), jnp.sin(ang)
        if j == 0:
            ca[0:64, :] = c[0:64]
            ca[64:128, :] = -s[0:64]
            ca[128:136, :] = jnp.where(rowi[0:8] == 0, alt[0:8], 0.0)
            ca[136:200, :] = c[64:128]
            ca[200:264, :] = -s[64:128]
            c2 = jnp.where(rowi == 0, c, 2.0 * c) * gscale
            s2 = jnp.where(rowi == 0, alt, -2.0 * s) * gscale
            cu[_C_G] = pack(blk2(jnp.where(first, c2, 0.0), jnp.where(first, 0.0, c2),
                                 jnp.where(first, s2, 0.0), jnp.where(first, 0.0, s2)))
        else:
            sg = jnp.where(first, -s, s)
            cg = jnp.where(first, -c, c)
            cu[_C_A + j - 1] = pack(blk2(c, sg, -s, cg))
            cu[_C_G + j] = pack(blk2(2.0 * gscale * c, -2.0 * gscale * sg, -2.0 * gscale * s, -2.0 * gscale * cg))
    ang = ((rowi * lane) & 127).astype(f32) * (2 * np.pi / 128)
    ca[264:392, :] = jnp.cos(ang)
    ca[392:520, :] = -jnp.sin(ang)
    tr[KR:, :] = jnp.zeros((640 - KR, S), f32)
    ti[KR:, :] = jnp.zeros((640 - KR, S), f32)

    def gen_ms(n1, carry):
        fr, fi = ca[264:392, :], ca[392:520, :]
        ang = (n1 * lane[0:8]).astype(f32) * (2 * np.pi / S)
        t_r = jnp.broadcast_to(jnp.cos(ang)[0:1], (128, 128))
        t_i = jnp.broadcast_to(-jnp.sin(ang)[0:1], (128, 128))
        mr, mi = fr * t_r - fi * t_i, fr * t_i + fi * t_r
        ms[n1] = pack(blk2(mr, mi, -mi, mr))
        return carry

    jax.lax.fori_loop(0, 16, gen_ms, 0)
    c_x[0].wait()

    def split_x(c, carry):
        r0 = pl.multiple_of(c * 128, 128)
        for a in range(8):
            xu[a, pl.ds(pl.multiple_of(c * 64, 64), 64), :] = pltpu.bitcast(ob[pl.ds(r0, 128), 128 * a:128 * (a + 1)], u32)
        return carry

    jax.lax.fori_loop(0, 8, split_x, 0)
    c_x[1].wait()
    jax.lax.fori_loop(8, 16, split_x, 0)

    def qkv_copy(t, p):
        w = (wq_hbm, wk_hbm, wv_hbm)[t]
        return pltpu.make_async_copy(w.bitcast(u32).at[:, p, :], wraw.at[t, p, 0:D], qsem.at[p])

    def fwd(i, carry):
        for k in range(2):
            for t in range(3):
                qkv_copy(t, (2 * i + k + 15) % 16).start()
        xw_t = [xu[a, pl.ds(i, 128, stride=8), :] for a in range(8)]
        for half in range(2):
            n1 = 2 * i + half
            x = [(_lo if half == 0 else _hi)(w) for w in xw_t]
            a0, a1, a2, a3 = x[0] + x[4], x[1] + x[5], x[2] + x[6], x[3] + x[7]
            d0, d1, d2, d3 = x[0] - x[4], x[1] - x[5], x[2] - x[6], x[3] - x[7]
            e0, e1 = a0 + a2, a1 + a3
            u, w = (d1 - d3) * _R2, (d1 + d3) * _R2
            p0, p4 = e0 + e1, e0 - e1
            planes = [(d0 + u, d2 + w), (a0 - a2, a1 - a3), (d0 - u, w - d2)]
            o0 = _dot_nt(ca[0:136, :], p0)
            o4 = _dot_nt(ca[136:264, :], p4)
            oj = [_dot_nt(cmat(_C_A + j), jnp.concatenate(planes[j], axis=1)) for j in range(3)]
            xr = jnp.concatenate([o0[0:64], o4[0:64]] + [o[0:128] for o in oj] + [o0[128:136]], axis=0)
            xi = jnp.concatenate([o0[64:128], o4[64:128]] + [o[128:256] for o in oj]
                                 + [jnp.zeros((8, 128), f32)], axis=0)
            t = _dot(jnp.concatenate([xr, xi], axis=1), pltpu.bitcast(ms[n1], bf16))
            c0 = pl.multiple_of(n1 * 128, 128)
            tr[0:KR, pl.ds(c0, 128)] = t[:, 0:128]
            ti[0:KR, pl.ds(c0, 128)] = t[:, 128:256]
        return carry

    jax.lax.fori_loop(0, 4, lambda i, c: fwd(2 * i + 1, fwd(2 * i, c)), 0)

    wait(c_w)

    def mid_group(r0, wr_fn, wi_fn):
        z = [(tr[pl.ds(r0, 8), 128 * n:128 * (n + 1)], ti[pl.ds(r0, 8), 128 * n:128 * (n + 1)]) for n in range(16)]
        z = _fft16(z, -1)
        q = []
        for k in range(16):
            wr, wi = wr_fn(k), wi_fn(k)
            zr, zi = z[k]
            q.append((zr * wr - zi * wi, zr * wi + zi * wr))
        z = _fft16(q, +1)
        for n in range(16):
            tr[pl.ds(r0, 8), 128 * n:128 * (n + 1)] = z[n][0]
            ti[pl.ds(r0, 8), 128 * n:128 * (n + 1)] = z[n][1]

    for blk, half, res in ((0, 0, 0), (0, 1, 4), (1, 0, 1), (1, 1, 7), (2, 0, 2), (2, 1, 6), (3, 0, 3), (3, 1, 5)):
        sel = _lo if res % 2 == 0 else _hi

        def mid(g, carry, blk=blk, half=half, res=res, sel=sel):
            r0 = pl.multiple_of(128 * blk + 64 * half + 8 * g, 8)
            p0 = res // 2 + 32 * g
            mid_group(r0,
                      lambda k: sel(wu[0, k, pl.ds(p0, 8, stride=4), :]),
                      lambda k: sel(wu[1, k, pl.ds(p0, 8, stride=4), :]))
            return carry

        jax.lax.fori_loop(0, 8, mid, 0)
    mid_group(512,
              lambda k: jnp.broadcast_to(wny[0, :, 128 * k:128 * (k + 1)].astype(f32), (8, 128)),
              lambda k: jnp.broadcast_to(wny[1, :, 128 * k:128 * (k + 1)].astype(f32), (8, 128)))

    def inv(i, carry):
        ys = []
        for half in range(2):
            n1 = 2 * i + half
            c0 = pl.multiple_of(n1 * 128, 128)
            mm = pltpu.bitcast(ms[n1], bf16)
            zc = jnp.concatenate([tr[0:512, pl.ds(c0, 128)], ti[0:512, pl.ds(c0, 128)]], axis=1)
            z = _dot_nt(mm, zc)
            zn = jnp.concatenate([tr[512:640, pl.ds(c0, 128)], ti[512:640, pl.ds(c0, 128)]], axis=1)
            ny = _dot_nt(mm[0:128], zn)
            zr, zi = z[0:128], z[128:256]
            zi0 = jnp.where(lane == 0, ny, zi[:, 0:128])
            u = _dot(jnp.concatenate([zr[:, 0:128], zi0], axis=1), cmat(_C_G))
            v = [_dot(jnp.concatenate([zr[:, 128 * j:128 * (j + 1)], zi[:, 128 * j:128 * (j + 1)]], axis=1),
                      cmat(_C_G + j)) for j in (1, 2, 3)]
            u0, u4 = u[:, 0:128], u[:, 128:256]
            v1r, v1i = v[0][:, 0:128], v[0][:, 128:256]
            v2r, v2i = v[1][:, 0:128], v[1][:, 128:256]
            v3r, v3i = v[2][:, 0:128], v[2][:, 128:256]
            e, o = u0 + u4, u0 - u4
            ep, em = e + v2r, e - v2r
            sa, da = v1r + v3r, v1r - v3r
            di, si = v1i - v3i, v1i + v3i
            p, q = (da - si) * _R2, (da + si) * _R2
            om, op = o - v2i, o + v2i
            ys.append([ep + sa, om + p, em - di, op - q, ep - sa, om - p, em + di, op + q])
        for a in range(8):
            bu[a, pl.ds(i, 128, stride=8), :] = (_bf16_word(ys[0][a]) >> 16) | _bf16_word(ys[1][a])
        return carry

    jax.lax.fori_loop(0, 4, lambda i, c: inv(2 * i + 1, inv(2 * i, c)), 0)

    wait(c_p)
    h_ref[0, 0:M, :] = mem0_ref[...].astype(f32)
    row = jax.lax.broadcasted_iota(i32, (L, L), 0)
    col = jax.lax.broadcasted_iota(i32, (L, L), 1)
    mask = (row < M) | (row >= col)
    scale = DH ** -0.5

    def load_x(s, hb):
        p0 = s * (SEG // 2) if isinstance(s, int) else pl.multiple_of(s * (SEG // 2), SEG // 2)
        for a in range(8):
            h_ref[hb, M:L, 128 * a:128 * (a + 1)] = pltpu.bitcast(xu[a, pl.ds(p0, SEG // 2), :], bf16).astype(f32)

    def probs(sc):
        sc = jnp.where(mask, sc * scale, -1e9)
        e = jnp.exp(sc - jnp.max(sc, axis=-1, keepdims=True))
        return e * (1.0 / jnp.sum(e, axis=-1, keepdims=True))

    def gate(hb):
        gw = gw_ref[...].astype(f32).reshape(1, D)
        return jax.nn.sigmoid(jnp.sum(h_ref[hb, M:L, :] * gw, axis=-1, keepdims=True))

    def finish(s, hn, j, r, g):
        r0 = s * SEG if isinstance(s, int) else pl.multiple_of(s * SEG, SEG)
        p0 = s * (SEG // 2) if isinstance(s, int) else pl.multiple_of(s * (SEG // 2), SEG // 2)
        c0 = j * 128
        h_ref[hn, 0:M, pl.ds(c0, 128)] = r[0:M]
        bb = pltpu.bitcast(bu[j, pl.ds(p0, SEG // 2), :], bf16).astype(f32)
        ob[pl.ds(r0, SEG), pl.ds(c0, 128)] = (bb + g * (r[M:L] - bb)).astype(bf16)

    def out_copy(s):
        r0 = s * SEG if isinstance(s, int) else pl.multiple_of(s * SEG, SEG)
        return pltpu.make_async_copy(ob.at[pl.ds(r0, SEG)], out_hbm.at[pl.ds(r0, SEG)], osem)

    def repack_wait(i):
        for t in range(3):
            qkv_copy(t, i).wait()

    def repack_body(i):
        for t in range(3):
            ev = wraw[t, i, pl.ds(0, 512, stride=2), :]
            od = wraw[t, i, pl.ds(1, 512, stride=2), :]
            wqkv[2 * i, :, 128 * t:128 * (t + 1)] = (ev & np.uint32(0xFFFF)) | (od << 16)
            wqkv[2 * i + 1, :, 128 * t:128 * (t + 1)] = (ev >> 16) | (od & np.uint32(0xFFFF0000))

    def repack(i, carry):
        repack_wait(i)
        repack_body(i)
        return carry

    repack(15, 0)
    wsp_ref[...] = wqkv[H - 1]

    def repack_pre(t, carry):
        @pl.when(t == 1)
        def _():
            start(c_o)

        for p in range(5):
            repack_wait(5 * t + p)
        for p in range(5):
            repack_body(5 * t + p)
        q0 = pl.multiple_of(16 + 336 * t, 16)
        xs = jnp.concatenate([pltpu.bitcast(xu[a, pl.ds(q0, 336), :], bf16) for a in range(8)], axis=1)
        xq = _dot(xs, pltpu.bitcast(wsp_ref[...], bf16))
        xq_ref[0, pl.ds(q0, 336), :] = pltpu.bitcast(xq.astype(bf16), u32)
        return carry

    jax.lax.fori_loop(0, 3, repack_pre, 0)
    load_x(0, 0)

    def step(s, hb, first):
        hn = (hb + 1) % UNROLL
        st = {}

        def qk(a):
            qkv = st[a]['qkv']
            st[a]['sc'] = _dot_nt(qkv[:, 0:128], qkv[:, 128:256])

        def softmax(a):
            st[a]['p'] = probs(st[a]['sc'])

        def pv(b):
            o_ref[:, b * 128:(b + 1) * 128] = _dot(st[b]['p'], st[b]['qkv'][:, 256:384])
            del st[b]

        for it in range(H):
            if it == H - 1 and not first:
                p0 = s * (SEG // 2) if isinstance(s, int) else pl.multiple_of(s * (SEG // 2), SEG // 2)
                xq = pltpu.bitcast(xq_ref[0, pl.ds(p0, SEG // 2), :], bf16).astype(f32)
                rm = _dot(h_ref[hb, 0:M, :], pltpu.bitcast(wqkv[it], bf16))
                st[it] = dict(qkv=jnp.concatenate([rm, xq], axis=0))
            elif it == 0:
                r = _dot(h_ref[hb, :, 0:512], pltpu.bitcast(wqkv[it, 0:256], bf16))
                st[it] = dict(qkv=_dot(h_ref[hb, :, 512:1024], pltpu.bitcast(wqkv[it, 256:512], bf16)) + r)
            else:
                st[it] = dict(qkv=_dot(h_ref[hb], pltpu.bitcast(wqkv[it], bf16)))
            if it >= LAGQ:
                qk(it - LAGQ)
            if it >= LAGP:
                pv(it - LAGP)
            if it >= LAGQ:
                softmax(it - LAGQ)
            if it == XAT:
                g = gate(hb)
                load_x(min(s + 1, NSEG - 1) if isinstance(s, int) else jnp.minimum(s + 1, NSEG - 1), hn)

        def wo_dot(j, h0, h1):
            w = wo2[j // 4, h0:h1, :, 128 * (j % 4):128 * (j % 4 + 1)]
            return _dot(o_ref[:, h0 * DH:h1 * DH], pltpu.bitcast(w.reshape((h1 - h0) * 64, 128), bf16))

        tail = []
        for t in range(LAGP):
            fns = []
            if t < LAGQ:
                fns.append(lambda a=H - LAGQ + t: qk(a))
            if t < LAGP - 1:
                fns.append(lambda b=H - LAGP + t: pv(b))
            if t < LAGQ:
                fns.append(lambda a=H - LAGQ + t: softmax(a))
            tail.append(fns)
        tail = tail[:max(LAGQ, LAGP - 1)] + [[], [lambda: pv(H - 1)]]
        npart = len(tail)
        assert npart == 4
        order = list(range(8 - npart, 8))
        if first:
            wait(c_o[0:4])
        for t, j in enumerate(order):
            part_ref[:, 128 * t:128 * (t + 1)] = wo_dot(j, 0, KS)
            for fn in tail[t]:
                fn()
        if first:
            wait(c_o[4:7])
            for j in range(4):
                part_ref[:, 128 * (4 + j):128 * (5 + j)] = wo_dot(j, 0, 24)
            c_o[7].wait()
            for j in range(4):
                finish(s, hn, j, part_ref[:, 128 * (4 + j):128 * (5 + j)] + wo_dot(j, 24, H), g)
        else:
            for j in range(8 - npart):
                finish(s, hn, j, wo_dot(j, 0, H), g)
        for t, j in enumerate(order):
            finish(s, hn, j, part_ref[:, 128 * t:128 * (t + 1)] + wo_dot(j, KS, H), g)
        out_copy(s).start()

    assert (NSEG - 1) % UNROLL == 0
    step(0, 0, True)

    def next_step(t, carry):
        for u in range(UNROLL):
            step(1 + t * UNROLL + u, (1 + u) % UNROLL, False)
        return carry

    jax.lax.fori_loop(0, (NSEG - 1) // UNROLL, next_step, 0)

    pltpu.make_async_copy(ob, out_hbm, osem).wait()


@functools.partial(jax.jit, static_argnames=("A_seg_len",))
def pallas_gated_mix__memory_aug_recurrent_mem_tr__spectral_gfnet__prompt_kernel(
    A_x, A_mem0, A_Wq, A_Wk, A_Wv, A_Wo, A_seg_len, B_x, B_w_r, B_w_i, gate_w,
):
    del B_x
    assert A_x.shape == (1, S, D) and A_mem0.shape == (1, M, D) and A_Wq.shape == (D, H, DH)
    assert int(A_seg_len) == SEG
    V = pltpu.VMEM
    hbm = pl.BlockSpec(memory_space=pltpu.MemorySpace.HBM)
    out = pl.pallas_call(
        _kernel,
        out_shape=jax.ShapeDtypeStruct((S, D), bf16),
        in_specs=[hbm] * 9,
        out_specs=hbm,
        scratch_shapes=[
            V((M, D), bf16),
            V((D,), bf16),
            V((8, S // 2 + 8, 128), u32),
            V((3, 16, D + 8, 128), u32),
            V((H, D // 2, 384), u32),
            V((2, H, DH // 2, 512), u32),
            V((7, 128, 256), u32),
            V((520, 128), f32),
            V((16, 128, 256), u32),
            V((2, 16, 256 + 8, 128), u32),
            V((2, 1, S), bf16),
            V((640, S), f32),
            V((640, S), f32),
            V((8, S // 2 + 8, 128), u32),
            V((UNROLL, L, D), f32),
            V((L, H * DH), f32),
            V((L, D), f32),
            V((1, S // 2, 384), u32),
            V((D // 2, 384), u32),
            V((S, D), bf16),
            pltpu.SemaphoreType.DMA((4,)),
            pltpu.SemaphoreType.DMA((16,)),
            pltpu.SemaphoreType.DMA((8,)),
            pltpu.SemaphoreType.DMA,
        ],
        compiler_params=pltpu.CompilerParams(vmem_limit_bytes=112 * 1024 * 1024),
    )(A_x.reshape(S, D), A_mem0.reshape(M, D), A_Wq, A_Wk, A_Wv, A_Wo,
      B_w_r.T, B_w_i.T, gate_w)
    return out.reshape(1, S, D)
```

```python
import functools

import jax
import jax.numpy as jnp
import numpy as np
import jax.experimental.pallas as pl
import jax.experimental.pallas.tpu as pltpu

f32 = jnp.float32
bf16 = jnp.bfloat16
u32 = jnp.uint32
i32 = jnp.int32

S, D, H, DH, M, SEG = 2048, 1024, 32, 128, 8, 32
L = M + SEG
NSEG = S // SEG
UNROLL = 3
LAGQ, LAGP = 1, 3
KS = 28
XAT = 8
NSP = 3
NPRE = (NSP + 1) // 2
WO_T = 1
KR = 520
_C_A, _C_G = 0, 3


def _dot(a, b):
    return jax.lax.dot_general(a, b, (((1,), (0,)), ((), ())), preferred_element_type=f32)


def _dot_nt(a, b):
    return jax.lax.dot_general(a, b, (((1,), (1,)), ((), ())), preferred_element_type=f32)


def _lo(w):
    return pltpu.bitcast(w << 16, f32)


def _hi(w):
    return pltpu.bitcast(w & np.uint32(0xFFFF0000), f32)


def _bf16_word(x):
    return pltpu.bitcast(x.astype(bf16).astype(f32), u32)


_R2 = float(np.sqrt(0.5))


def _cmul_const(z, ang):
    zr, zi = z
    c, s = float(np.cos(ang)), float(np.sin(ang))
    q = int(round(ang / (np.pi / 4)))
    if abs(ang - q * np.pi / 4) < 1e-9:
        q %= 8
        if q == 0:
            return zr, zi
        if q == 2:
            return -zi, zr
        if q == 4:
            return -zr, -zi
        if q == 6:
            return zi, -zr
        if q == 1:
            return (zr - zi) * _R2, (zr + zi) * _R2
        if q == 3:
            return (zr + zi) * (-_R2), (zr - zi) * _R2
        if q == 5:
            return (zi - zr) * _R2, (zr + zi) * (-_R2)
        return (zr + zi) * _R2, (zi - zr) * _R2
    return zr * c - zi * s, zr * s + zi * c


def _add(a, b):
    return a[0] + b[0], a[1] + b[1]


def _sub(a, b):
    return a[0] - b[0], a[1] - b[1]


def _bfly4(x0, x1, x2, x3, sign):
    s0, s1 = _add(x0, x2), _sub(x0, x2)
    s2, s3 = _add(x1, x3), _sub(x1, x3)
    y0, y2 = _add(s0, s2), _sub(s0, s2)
    if sign < 0:
        y1 = (s1[0] + s3[1], s1[1] - s3[0])
        y3 = (s1[0] - s3[1], s1[1] + s3[0])
    else:
        y1 = (s1[0] - s3[1], s1[1] + s3[0])
        y3 = (s1[0] + s3[1], s1[1] - s3[0])
    return y0, y1, y2, y3


def _fft16(x, sign):
    t = [[None] * 4 for _ in range(4)]
    for b in range(4):
        y = _bfly4(x[b], x[4 + b], x[8 + b], x[12 + b], sign)
        for c in range(4):
            t[c][b] = _cmul_const(y[c], sign * 2 * np.pi * b * c / 16)
    out = [None] * 16
    for c in range(4):
        y = _bfly4(t[c][0], t[c][1], t[c][2], t[c][3], sign)
        for d in range(4):
            out[c + 4 * d] = y[d]
    return out


def _kernel(x_hbm, mem0_hbm, wq_hbm, wk_hbm, wv_hbm, wo_hbm, wrt_hbm, wit_hbm, gw_hbm,
            out_hbm,
            mem0_ref, gw_ref, xu, wraw, wqkv, wo2, cu, ca, ms, wu, wny, tr, ti, bu, h_ref, o_ref, part_ref, xq_ref, wsp_ref, ob, sems, qsem, wsem, osem):
    def start(cs):
        for c in cs:
            c.start()

    def wait(cs):
        for c in cs:
            c.wait()

    c_x = [pltpu.make_async_copy(x_hbm.at[1024 * c:1024 * c + 1024], ob.at[1024 * c:1024 * c + 1024], sems.at[3 * c])
           for c in range(2)]
    c_w = []
    for t, w in enumerate((wrt_hbm, wit_hbm)):
        ww = w.at[0:512].bitcast(u32)
        c_w += [pltpu.make_async_copy(ww.at[:, 128 * k:128 * (k + 1)], wu.at[t, k, 0:256], sems.at[1]) for k in range(16)]
        c_w.append(pltpu.make_async_copy(w.at[512:513], wny.at[t], sems.at[1]))
    wow = wo_hbm.bitcast(u32)
    c_o = [pltpu.make_async_copy(wow.at[8 * q:8 * q + 8, :, 512 * hf:512 * (hf + 1)], wo2.at[hf, 8 * q:8 * q + 8],
                                 wsem.at[4 * hf + q]) for hf in (1, 0) for q in range(4)]
    c_p = [pltpu.make_async_copy(mem0_hbm, mem0_ref, sems.at[2]), pltpu.make_async_copy(gw_hbm, gw_ref, sems.at[2])]
    start(c_x)
    start(c_p)
    start(c_w)

    lane = jax.lax.broadcasted_iota(i32, (128, 128), 1)

    def cmat(i):
        return pltpu.bitcast(cu[i], bf16)

    rowi = jax.lax.broadcasted_iota(i32, (128, 128), 0)
    first = rowi < 64
    gscale = 1.0 / (D * S)

    def pack(m):
        return pltpu.bitcast(m.astype(bf16), u32)

    def blk2(a, b, c, d):
        return jnp.concatenate([jnp.concatenate([a, b], axis=1), jnp.concatenate([c, d], axis=1)], axis=0)

    alt = jnp.where((lane & 1) == 0, 1.0, -1.0).astype(f32)
    for j in range(4):
        lo, hi = (0, 4) if j == 0 else (j, 8 - j)
        k = jnp.where(first, lo + 8 * rowi, hi + 8 * (rowi - 64))
        ang = ((k * lane) & (D - 1)).astype(f32) * (2 * np.pi / D)
        c, s = jnp.cos(ang), jnp.sin(ang)
        if j == 0:
            ca[0:64, :] = c[0:64]
            ca[64:128, :] = -s[0:64]
            ca[128:136, :] = jnp.where(rowi[0:8] == 0, alt[0:8], 0.0)
            ca[136:200, :] = c[64:128]
            ca[200:264, :] = -s[64:128]
            c2 = jnp.where(rowi == 0, c, 2.0 * c) * gscale
            s2 = jnp.where(rowi == 0, alt, -2.0 * s) * gscale
            cu[_C_G] = pack(blk2(jnp.where(first, c2, 0.0), jnp.where(first, 0.0, c2),
                                 jnp.where(first, s2, 0.0), jnp.where(first, 0.0, s2)))
        else:
            sg = jnp.where(first, -s, s)
            cg = jnp.where(first, -c, c)
            cu[_C_A + j - 1] = pack(blk2(c, sg, -s, cg))
            cu[_C_G + j] = pack(blk2(2.0 * gscale * c, -2.0 * gscale * sg, -2.0 * gscale * s, -2.0 * gscale * cg))
    ang = ((rowi * lane) & 127).astype(f32) * (2 * np.pi / 128)
    ca[264:392, :] = jnp.cos(ang)
    ca[392:520, :] = -jnp.sin(ang)
    tr[KR:, :] = jnp.zeros((640 - KR, S), f32)
    ti[KR:, :] = jnp.zeros((640 - KR, S), f32)

    def gen_ms(n1, carry):
        fr, fi = ca[264:392, :], ca[392:520, :]
        ang = (n1 * lane[0:8]).astype(f32) * (2 * np.pi / S)
        t_r = jnp.broadcast_to(jnp.cos(ang)[0:1], (128, 128))
        t_i = jnp.broadcast_to(-jnp.sin(ang)[0:1], (128, 128))
        mr, mi = fr * t_r - fi * t_i, fr * t_i + fi * t_r
        ms[n1] = pack(blk2(mr, mi, -mi, mr))
        return carry

    jax.lax.fori_loop(0, 16, gen_ms, 0)
    c_x[0].wait()

    def split_x(c, carry):
        r0 = pl.multiple_of(c * 128, 128)
        for a in range(8):
            xu[a, pl.ds(pl.multiple_of(c * 64, 64), 64), :] = pltpu.bitcast(ob[pl.ds(r0, 128), 128 * a:128 * (a + 1)], u32)
        return carry

    jax.lax.fori_loop(0, 8, split_x, 0)
    c_x[1].wait()
    jax.lax.fori_loop(8, 16, split_x, 0)

    def qkv_copy(t, p):
        w = (wq_hbm, wk_hbm, wv_hbm)[t]
        return pltpu.make_async_copy(w.bitcast(u32).at[:, p, :], wraw.at[t, p, 0:D], qsem.at[p])

    def fwd(i, carry):
        for k in range(2):
            for t in range(3):
                qkv_copy(t, (2 * i + k + 14) % 16).start()
        xw_t = [xu[a, pl.ds(i, 128, stride=8), :] for a in range(8)]
        for half in range(2):
            n1 = 2 * i + half
            x = [(_lo if half == 0 else _hi)(w) for w in xw_t]
            a0, a1, a2, a3 = x[0] + x[4], x[1] + x[5], x[2] + x[6], x[3] + x[7]
            d0, d1, d2, d3 = x[0] - x[4], x[1] - x[5], x[2] - x[6], x[3] - x[7]
            e0, e1 = a0 + a2, a1 + a3
            u, w = (d1 - d3) * _R2, (d1 + d3) * _R2
            p0, p4 = e0 + e1, e0 - e1
            planes = [(d0 + u, d2 + w), (a0 - a2, a1 - a3), (d0 - u, w - d2)]
            o0 = _dot_nt(ca[0:136, :], p0)
            o4 = _dot_nt(ca[136:264, :], p4)
            oj = [_dot_nt(cmat(_C_A + j), jnp.concatenate(planes[j], axis=1)) for j in range(3)]
            xr = jnp.concatenate([o0[0:64], o4[0:64]] + [o[0:128] for o in oj] + [o0[128:136]], axis=0)
            xi = jnp.concatenate([o0[64:128], o4[64:128]] + [o[128:256] for o in oj]
                                 + [jnp.zeros((8, 128), f32)], axis=0)
            t = _dot(jnp.concatenate([xr, xi], axis=1), pltpu.bitcast(ms[n1], bf16))
            c0 = pl.multiple_of(n1 * 128, 128)
            tr[0:KR, pl.ds(c0, 128)] = t[:, 0:128]
            ti[0:KR, pl.ds(c0, 128)] = t[:, 128:256]
        return carry

    jax.lax.fori_loop(0, 4, lambda i, c: fwd(2 * i + 1, fwd(2 * i, c)), 0)

    wait(c_w)

    def mid_group(r0, wr_fn, wi_fn):
        z = [(tr[pl.ds(r0, 8), 128 * n:128 * (n + 1)], ti[pl.ds(r0, 8), 128 * n:128 * (n + 1)]) for n in range(16)]
        z = _fft16(z, -1)
        q = []
        for k in range(16):
            wr, wi = wr_fn(k), wi_fn(k)
            zr, zi = z[k]
            q.append((zr * wr - zi * wi, zr * wi + zi * wr))
        z = _fft16(q, +1)
        for n in range(16):
            tr[pl.ds(r0, 8), 128 * n:128 * (n + 1)] = z[n][0]
            ti[pl.ds(r0, 8), 128 * n:128 * (n + 1)] = z[n][1]

    for blk, half, res in ((0, 0, 0), (0, 1, 4), (1, 0, 1), (1, 1, 7), (2, 0, 2), (2, 1, 6), (3, 0, 3), (3, 1, 5)):
        sel = _lo if res % 2 == 0 else _hi

        def mid(g, carry, blk=blk, half=half, res=res, sel=sel):
            r0 = pl.multiple_of(128 * blk + 64 * half + 8 * g, 8)
            p0 = res // 2 + 32 * g
            mid_group(r0,
                      lambda k: sel(wu[0, k, pl.ds(p0, 8, stride=4), :]),
                      lambda k: sel(wu[1, k, pl.ds(p0, 8, stride=4), :]))
            return carry

        jax.lax.fori_loop(0, 8, mid, 0)
    mid_group(512,
              lambda k: jnp.broadcast_to(wny[0, :, 128 * k:128 * (k + 1)].astype(f32), (8, 128)),
              lambda k: jnp.broadcast_to(wny[1, :, 128 * k:128 * (k + 1)].astype(f32), (8, 128)))

    def inv(i, carry):
        ys = []
        for half in range(2):
            n1 = 2 * i + half
            c0 = pl.multiple_of(n1 * 128, 128)
            mm = pltpu.bitcast(ms[n1], bf16)
            zc = jnp.concatenate([tr[0:512, pl.ds(c0, 128)], ti[0:512, pl.ds(c0, 128)]], axis=1)
            z = _dot_nt(mm, zc)
            zn = jnp.concatenate([tr[512:640, pl.ds(c0, 128)], ti[512:640, pl.ds(c0, 128)]], axis=1)
            ny = _dot_nt(mm[0:128], zn)
            zr, zi = z[0:128], z[128:256]
            zi0 = jnp.where(lane == 0, ny, zi[:, 0:128])
            u = _dot(jnp.concatenate([zr[:, 0:128], zi0], axis=1), cmat(_C_G))
            v = [_dot(jnp.concatenate([zr[:, 128 * j:128 * (j + 1)], zi[:, 128 * j:128 * (j + 1)]], axis=1),
                      cmat(_C_G + j)) for j in (1, 2, 3)]
            u0, u4 = u[:, 0:128], u[:, 128:256]
            v1r, v1i = v[0][:, 0:128], v[0][:, 128:256]
            v2r, v2i = v[1][:, 0:128], v[1][:, 128:256]
            v3r, v3i = v[2][:, 0:128], v[2][:, 128:256]
            e, o = u0 + u4, u0 - u4
            ep, em = e + v2r, e - v2r
            sa, da = v1r + v3r, v1r - v3r
            di, si = v1i - v3i, v1i + v3i
            p, q = (da - si) * _R2, (da + si) * _R2
            om, op = o - v2i, o + v2i
            ys.append([ep + sa, om + p, em - di, op - q, ep - sa, om - p, em + di, op + q])
        for a in range(8):
            bu[a, pl.ds(i, 128, stride=8), :] = (_bf16_word(ys[0][a]) >> 16) | _bf16_word(ys[1][a])
        return carry

    jax.lax.fori_loop(0, 4, lambda i, c: inv(2 * i + 1, inv(2 * i, c)), 0)

    wait(c_p)
    h_ref[0, 0:M, :] = mem0_ref[...].astype(f32)
    row = jax.lax.broadcasted_iota(i32, (L, L), 0)
    col = jax.lax.broadcasted_iota(i32, (L, L), 1)
    mask = (row < M) | (row >= col)
    scale = DH ** -0.5

    def load_x(s, hb):
        p0 = s * (SEG // 2) if isinstance(s, int) else pl.multiple_of(s * (SEG // 2), SEG // 2)
        for a in range(8):
            h_ref[hb, M:L, 128 * a:128 * (a + 1)] = pltpu.bitcast(xu[a, pl.ds(p0, SEG // 2), :], bf16).astype(f32)

    def probs(sc):
        sc = jnp.where(mask, sc * scale, -1e9)
        e = jnp.exp(sc - jnp.max(sc, axis=-1, keepdims=True))
        return e * (1.0 / jnp.sum(e, axis=-1, keepdims=True))

    def gate(hb):
        gw = gw_ref[...].astype(f32).reshape(1, D)
        return jax.nn.sigmoid(jnp.sum(h_ref[hb, M:L, :] * gw, axis=-1, keepdims=True))

    def finish(s, hn, j, r, g):
        r0 = s * SEG if isinstance(s, int) else pl.multiple_of(s * SEG, SEG)
        p0 = s * (SEG // 2) if isinstance(s, int) else pl.multiple_of(s * (SEG // 2), SEG // 2)
        c0 = j * 128
        h_ref[hn, 0:M, pl.ds(c0, 128)] = r[0:M]
        bb = pltpu.bitcast(bu[j, pl.ds(p0, SEG // 2), :], bf16).astype(f32)
        ob[pl.ds(r0, SEG), pl.ds(c0, 128)] = (bb + g * (r[M:L] - bb)).astype(bf16)

    def out_copy(s):
        r0 = s * SEG if isinstance(s, int) else pl.multiple_of(s * SEG, SEG)
        return pltpu.make_async_copy(ob.at[pl.ds(r0, SEG)], out_hbm.at[pl.ds(r0, SEG)], osem)

    def repack_wait(i):
        for t in range(3):
            qkv_copy(t, i).wait()

    def repack_body(i):
        for t in range(3):
            ev = wraw[t, i, pl.ds(0, 512, stride=2), :]
            od = wraw[t, i, pl.ds(1, 512, stride=2), :]
            wqkv[2 * i, :, 128 * t:128 * (t + 1)] = (ev & np.uint32(0xFFFF)) | (od << 16)
            wqkv[2 * i + 1, :, 128 * t:128 * (t + 1)] = (ev >> 16) | (od & np.uint32(0xFFFF0000))

    for i in range(16 - NPRE, 16):
        repack_wait(i)
    for n in range(NSP):
        hd = H - NSP + n
        for t in range(3):
            ev = wraw[t, hd // 2, pl.ds(0, 512, stride=2), :]
            od = wraw[t, hd // 2, pl.ds(1, 512, stride=2), :]
            wsp_ref[:, 384 * n + 128 * t:384 * n + 128 * (t + 1)] = (
                (ev & np.uint32(0xFFFF)) | (od << 16) if hd % 2 == 0
                else (ev >> 16) | (od & np.uint32(0xFFFF0000)))

    def repack_pre(t, carry):
        @pl.when(t == WO_T)
        def _():
            start(c_o)

        for p in range(4 - NPRE):
            repack_wait(4 * t + p)

        @pl.when(t < 3)
        def _():
            for p in range(4 - NPRE, 4):
                repack_wait(4 * t + p)

        xs = jnp.concatenate(
            [ob[pl.ds(pl.multiple_of((16 * t + m) * SEG + SEG - 8, 8), 8), :] for m in range(16)], axis=0)
        xq_ref[pl.ds(pl.multiple_of(128 * t, 128), 128), :] = _dot(xs, pltpu.bitcast(wsp_ref[...], bf16))
        for p in range(4):
            repack_body(4 * t + p)
        return carry

    jax.lax.fori_loop(0, 4, repack_pre, 0)
    load_x(0, 0)

    def step(s, hb, first):
        hn = (hb + 1) % UNROLL
        st = {}

        def qk(a):
            qkv = st[a]['qkv']
            st[a]['sc'] = _dot_nt(qkv[:, 0:128], qkv[:, 128:256])

        def softmax(a):
            st[a]['p'] = probs(st[a]['sc'])

        def pv(b):
            o_ref[:, b * 128:(b + 1) * 128] = _dot(st[b]['p'], st[b]['qkv'][:, 256:384])
            del st[b]

        for it in range(H):
            if it >= H - NSP:
                c0 = 384 * (it - (H - NSP))
                xq = xq_ref[pl.ds(s * 8 if isinstance(s, int) else pl.multiple_of(s * 8, 8), 8), c0:c0 + 384]
                st[it] = dict(qkv=jnp.concatenate([_dot(h_ref[hb, 0:L - 8, :], pltpu.bitcast(wqkv[it], bf16)), xq], axis=0))
            elif it == 0:
                r = _dot(h_ref[hb, :, 0:512], pltpu.bitcast(wqkv[it, 0:256], bf16))
                st[it] = dict(qkv=_dot(h_ref[hb, :, 512:1024], pltpu.bitcast(wqkv[it, 256:512], bf16)) + r)
            else:
                st[it] = dict(qkv=_dot(h_ref[hb], pltpu.bitcast(wqkv[it], bf16)))
            if it >= LAGQ:
                qk(it - LAGQ)
            if it >= LAGP:
                pv(it - LAGP)
            if it >= LAGQ:
                softmax(it - LAGQ)
            if it == XAT:
                g = gate(hb)
                load_x(min(s + 1, NSEG - 1) if isinstance(s, int) else jnp.minimum(s + 1, NSEG - 1), hn)

        def wo_dot(j, h0, h1):
            w = wo2[j // 4, h0:h1, :, 128 * (j % 4):128 * (j % 4 + 1)]
            return _dot(o_ref[:, h0 * DH:h1 * DH], pltpu.bitcast(w.reshape((h1 - h0) * 64, 128), bf16))

        tail = []
        for t in range(LAGP):
            fns = []
            if t < LAGQ:
                fns.append(lambda a=H - LAGQ + t: qk(a))
            if t < LAGP - 1:
                fns.append(lambda b=H - LAGP + t: pv(b))
            if t < LAGQ:
                fns.append(lambda a=H - LAGQ + t: softmax(a))
            tail.append(fns)
        tail = tail[:max(LAGQ, LAGP - 1)] + [[], [lambda: pv(H - 1)]]
        npart = len(tail)
        assert npart == 4
        order = list(range(8 - npart, 8))
        if first:
            wait(c_o[0:4])
        for t, j in enumerate(order):
            part_ref[:, 128 * t:128 * (t + 1)] = wo_dot(j, 0, KS)
            for fn in tail[t]:
                fn()
        if first:
            wait(c_o[4:7])
            for j in range(4):
                part_ref[:, 128 * (4 + j):128 * (5 + j)] = wo_dot(j, 0, 24)
            c_o[7].wait()
            for j in range(4):
                finish(s, hn, j, part_ref[:, 128 * (4 + j):128 * (5 + j)] + wo_dot(j, 24, H), g)
        else:
            for j in range(8 - npart):
                finish(s, hn, j, wo_dot(j, 0, H), g)
        for t, j in enumerate(order):
            finish(s, hn, j, part_ref[:, 128 * t:128 * (t + 1)] + wo_dot(j, KS, H), g)
        out_copy(s).start()

    assert (NSEG - 1) % UNROLL == 0
    step(0, 0, True)

    def next_step(t, carry):
        for u in range(UNROLL):
            step(1 + t * UNROLL + u, (1 + u) % UNROLL, False)
        return carry

    jax.lax.fori_loop(0, (NSEG - 1) // UNROLL, next_step, 0)

    pltpu.make_async_copy(ob, out_hbm, osem).wait()


@functools.partial(jax.jit, static_argnames=("A_seg_len",))
def pallas_gated_mix__memory_aug_recurrent_mem_tr__spectral_gfnet__prompt_kernel(
    A_x, A_mem0, A_Wq, A_Wk, A_Wv, A_Wo, A_seg_len, B_x, B_w_r, B_w_i, gate_w,
):
    del B_x
    assert A_x.shape == (1, S, D) and A_mem0.shape == (1, M, D) and A_Wq.shape == (D, H, DH)
    assert int(A_seg_len) == SEG
    V = pltpu.VMEM
    hbm = pl.BlockSpec(memory_space=pltpu.MemorySpace.HBM)
    out = pl.pallas_call(
        _kernel,
        out_shape=jax.ShapeDtypeStruct((S, D), bf16),
        in_specs=[hbm] * 9,
        out_specs=hbm,
        scratch_shapes=[
            V((M, D), bf16),
            V((D,), bf16),
            V((8, S // 2 + 8, 128), u32),
            V((3, 16, D + 8, 128), u32),
            V((H, D // 2, 384), u32),
            V((2, H, DH // 2, 512), u32),
            V((7, 128, 256), u32),
            V((520, 128), f32),
            V((16, 128, 256), u32),
            V((2, 16, 256 + 8, 128), u32),
            V((2, 1, S), bf16),
            V((640, S), f32),
            V((640, S), f32),
            V((8, S // 2 + 8, 128), u32),
            V((UNROLL, L, D), f32),
            V((L, H * DH), f32),
            V((L, D), f32),
            V((NSEG * 8, NSP * 384), f32),
            V((D // 2, NSP * 384), u32),
            V((S, D), bf16),
            pltpu.SemaphoreType.DMA((4,)),
            pltpu.SemaphoreType.DMA((16,)),
            pltpu.SemaphoreType.DMA((8,)),
            pltpu.SemaphoreType.DMA,
        ],
        compiler_params=pltpu.CompilerParams(vmem_limit_bytes=112 * 1024 * 1024),
    )(A_x.reshape(S, D), A_mem0.reshape(M, D), A_Wq, A_Wk, A_Wv, A_Wo,
      B_w_r.T, B_w_i.T, gate_w)
    return out.reshape(1, S, D)
```
